```python
import os as _os
_os.environ.setdefault("JAX_PLATFORMS", "cpu")
import jax
import jax.numpy as jnp

def _softmax(x, axis=-1):
    return jax.nn.softmax(x, axis=axis)
def _gelu(x):
    return jax.nn.gelu(x, approximate=True)
def _silu(x):
    return jax.nn.silu(x)
def _sigmoid(x):
    return jax.nn.sigmoid(x)
def _layernorm(x, axis=-1, eps=1e-5):
    m = jnp.mean(x, axis=axis, keepdims=True)
    v = jnp.var(x, axis=axis, keepdims=True)
    return (x - m) / jnp.sqrt(v + eps)
def _scatter_add(tgt, idx, src, axis=0):
    return tgt.at[idx].add(src)
def _segment_sum(src, seg, n):
    return jax.ops.segment_sum(src, seg, n)
class _Rng:
    def __init__(self, key):
        self._k = key
    def _next(self):
        self._k, sub = jax.random.split(self._k)
        return sub
    def normal(self, shape):
        return jax.random.normal(self._next(), shape, dtype=jnp.bfloat16)
    def randint(self, lo, hi, shape):
        return jax.random.randint(self._next(), shape, lo, hi, dtype=jnp.int32)
    def uniform(self, shape, lo=0.0, hi=1.0):
        return jax.random.uniform(self._next(), shape, jnp.bfloat16, lo, hi)
    def permutation(self, n):
        return jax.random.permutation(self._next(), n)


kernel_name = 'sequential_preLN__ssm_conv_h3__dense_activation_gelu__prompt'

def setup_inputs():
    _rng = _Rng(jax.random.key(int.from_bytes(__import__("os").urandom(4), "little")))
    _w = (lambda a: (lambda t: t.astype(jnp.bfloat16) if jnp.issubdtype(t.dtype, jnp.floating) else t)(jnp.asarray(a)))
    def _A_setup():
        B, S, D = 1, 2048, 512
        ks = 4
        return {
            "q": _w((lambda *s: _rng.normal(s) * 0.05)(B, S, D)),
            "k": _w((lambda *s: _rng.normal(s) * 0.2)(B, S, D)),
            "v": _w((lambda *s: _rng.normal(s) * 0.2)(B, S, D)),
            "shift_k": _w((lambda *s: _rng.normal(s) * 0.2)(D, ks) * 0.5),
            "ssm_k": _w((lambda *s: _rng.normal(s) * 0.2)(D, S) * (1.0 / S ** 0.5)),
            "ssm_D": _w((lambda *s: _rng.normal(s) * 0.2)(D)),
        }
    _A_in = _A_setup()

    def _B_setup():
        B, S, D, F = 1, 2048, 512, 1376
        return {
            "x": _w((lambda *s: _rng.normal(s) * 0.05)(B, S, D)),
            "w1": _w((lambda *s: _rng.normal(s) * 0.2)(D, F) * (D ** -0.5)),
            "b1": _w((lambda *s: _rng.normal(s) * 0.2)(F) * 0.01),
            "w2": _w((lambda *s: _rng.normal(s) * 0.2)(F, D) * (F ** -0.5)),
            "b2": _w((lambda *s: _rng.normal(s) * 0.05)(D) * 0.01),
        }
    _B_in = _B_setup()

    return {
        "A_q": _A_in["q"],
        "A_k": _A_in["k"],
        "A_v": _A_in["v"],
        "A_shift_k": _A_in["shift_k"],
        "A_ssm_k": _A_in["ssm_k"],
        "A_ssm_D": _A_in["ssm_D"],
        "B_x": _B_in["x"],
        "B_w1": _B_in["w1"],
        "B_b1": _B_in["b1"],
        "B_w2": _B_in["w2"],
        "B_b2": _B_in["b2"],
    }

def reference(A_q, A_k, A_v, A_shift_k, A_ssm_k, A_ssm_D, B_x, B_w1, B_b1, B_w2, B_b2):
    def _A_ref(q, k, v, shift_k, ssm_k, ssm_D):
        B, S, D = q.shape
        ks = shift_k.shape[-1]
        k_pad = jnp.pad(k, ((0, 0), (ks - 1, 0), (0, 0)))
        k_shift = jnp.zeros_like(k)
        for t in range(ks):
            k_shift = k_shift + k_pad[:, t:t + S, :] * shift_k[:, ks - 1 - t][None, None, :]
        kv = k_shift * v
        L = 2 * S
        kv_pad = jnp.pad(kv, ((0, 0), (0, S), (0, 0)))
        kf_pad = jnp.pad(ssm_k, ((0, 0), (0, S)))
        kv_f = (lambda x, axes=(-2,-1): jnp.fft.rfft2(x.astype(jnp.float32), axes=axes))(kv_pad[:, None, :, :], axes=(1, 2))
        kf_f = (lambda x, axes=(-2,-1): jnp.fft.rfft2(x.astype(jnp.float32), axes=axes))(kf_pad[:, None, :], axes=(1, 2))
        kf_f = (lambda x, *d: x.transpose(*d))(kf_f, 1, 2, 0)
        y_f = kv_f * kf_f[None, :, :, :]
        y = (lambda x, s, axes=(-2,-1): jnp.fft.irfft2(x, s=s, axes=axes).astype(jnp.bfloat16))(y_f, (1, L), axes=(1, 2))[:, 0, :S, :]
        y = y + kv * ssm_D[None, None, :]
        return q * y

    def _B_ref(x, w1, b1, w2, b2):
        h = jnp.einsum("bsd,df->bsf", x, w1) + b1
        h = _gelu(h)
        return jnp.einsum("bsf,fd->bsd", h, w2) + b2

    x = A_q
    h = x + _A_ref(_layernorm(x, axis=-1), A_k, A_v, A_shift_k, A_ssm_k, A_ssm_D)
    h2 = h + _B_ref(_layernorm(h, axis=-1), B_w1, B_b1, B_w2, B_b2)
    return h2
```

```python
import functools
import numpy as np
import ml_dtypes
import jax
import jax.numpy as jnp
import jax.experimental.pallas as pl
import jax.experimental.pallas.tpu as pltpu

S, D, F = 2048, 512, 1376
B = 128
NB = S // B
TM = 256
NS = S // TM
LT = D // 128
GR = 16
NG = B // GR
EPS = 1e-5
NT = (((1,), (1,)), ((), ()))
PR = B + 8
FC = [(0, 512), (512, 1024), (1024, F)]
GELU_C = float(np.sqrt(2.0 / np.pi))
HCAP = 300.0

ASSIGN = {
    0: ([], []),
    1: ([(0, 1)], [[(1, 2)]]),
    2: ([(0, 2)], [[(1, 3), (2, 3)], [(2, 4)]]),
    3: ([(0, 3)], [[(0, 4), (1, 4)], [(0, 5), (1, 5), (2, 5)]]),
    4: ([(3, 4)], [[(3, 5)], [(0, 6), (1, 6), (2, 6)]]),
    5: ([(4, 5)], [[(3, 6)], [(0, 7), (1, 7)]]),
    6: ([(4, 6), (5, 6)], [[(2, 7), (3, 7)]]),
    7: ([(5, 7), (6, 7)], [[(4, 7)]]),
}


def _pack_rows(a):
    b = np.asarray(a, dtype=ml_dtypes.bfloat16).view(np.uint16).astype(np.uint32)
    return b[0::2] | (b[1::2] << 16)


def _consts():
    k = np.concatenate([np.arange(0, B, 2), np.arange(1, B, 2)]).astype(np.float64)
    n = np.arange(B, dtype=np.float64)
    th = 2.0 * np.pi * (k[:, None] + 0.5) / (2 * B)

    def fwd(shift):
        ang = th * (n[None, :] - shift)
        re = np.cos(ang).reshape(NG, GR, B)
        im = -np.sin(ang).reshape(NG, GR, B)
        return np.stack([re, im], axis=1).reshape(2 * B, B)
    fx = fwd(0.0)
    fh = fwd((B - 1) / 2.0)
    m = np.arange(B // 2, dtype=np.float64) + 0.5
    ci = np.cos(th * m[None, :]).T / B
    si = np.sin(th * m[None, :]).T / B
    return np.concatenate([_pack_rows(fx), _pack_rows(fh), _pack_rows(ci), _pack_rows(si)], axis=0)


def _kernel(flag_hbm, tab_hbm, q_hbm, k_hbm, v_hbm, sk_hbm, h_hbm, dvec_hbm, w1_hbm, b1_hbm, w2_hbm, b2_hbm,
            o_hbm,
            flag, tab, skv, dvv, b1v, b2v, qb, kb, vb, hb, w1b, w2b, w1p, w2p, ob, k32, skb,
            xs, gs, zacc, kvp, hres, xnp, zp, ybuf, gb0, gb1, gb2, acc0, acc1, st_m, st_r, st_m2, st_r2, xcb, sems):
    f32 = jnp.float32
    bf16 = jnp.bfloat16
    u32 = jnp.uint32
    P = functools.partial

    def rows(i):
        return pl.ds(i * TM, TM)

    def hcp(i):
        return (h_hbm.at[:, pl.ds(i * TM, TM)], hb.at[:, pl.ds(i * TM, TM)])

    def kcp(i):
        return (k_hbm.at[rows(i)], kb.at[rows(i)])

    def vcp(i):
        return (v_hbm.at[rows(i)], vb.at[rows(i)])

    def qcp(i):
        return (q_hbm.at[rows(i)], qb.at[rows(i)])

    def wcp(src, dst, c):
        lo, hi = FC[c]
        return (src.at[pl.ds(lo, hi - lo)], dst.at[pl.ds(lo, hi - lo)])

    groups = [
        ("a", [kcp(0), vcp(0), (sk_hbm, skv), (tab_hbm.at[pl.ds(0, 128)], tab.at[pl.ds(0, 128)])]),
        ("b", [(tab_hbm.at[pl.ds(128, 192)], tab.at[pl.ds(128, 192)]), hcp(0), (dvec_hbm, dvv)]),
        ("q0", [qcp(0)]),
        ("w1c0", [(b1_hbm, b1v), wcp(w1_hbm, w1b, 0)]),
        ("c", [hcp(1), kcp(1), vcp(1)]),
        ("w1c1", [wcp(w1_hbm, w1b, 1), qcp(1)]),
        ("w2c0", [(b2_hbm, b2v), wcp(w2_hbm, w2b, 0)]),
        ("w1c2", [wcp(w1_hbm, w1b, 2)]),
        ("w2c1", [wcp(w2_hbm, w2b, 1), wcp(w2_hbm, w2b, 2)]),
        ("d", [kcp(2), vcp(2), hcp(2), qcp(2)]),
        ("e", [kcp(3), vcp(3), hcp(3), hcp(4), hcp(5), kcp(4)]),
        ("f", [qcp(3), vcp(4), hcp(6), hcp(7), kcp(5)]),
        ("g", [qcp(4), vcp(5), qcp(5), kcp(6), vcp(6), qcp(6), kcp(7), vcp(7), qcp(7)]),
    ]
    cps = {name: [pltpu.make_async_copy(s, d, sems.at[gi]) for s, d in lst] for gi, (name, lst) in enumerate(groups)}
    nsem = len(groups)
    cp_flag = pltpu.make_async_copy(flag_hbm, flag, sems.at[nsem])
    cp_o = [pltpu.make_async_copy(ob.at[rows(i)], o_hbm.at[rows(i)], sems.at[nsem + 1]) for i in range(NS)]

    def wait(name):
        for c in cps[name]:
            c.wait()

    cp_flag.start()
    for name, _ in groups:
        for c in cps[name]:
            c.start()
    cp_flag.wait()
    pred = flag[15] != 0
    zero = flag[14]

    def drow(start, n):
        return pl.ds(pl.multiple_of(zero + start, 8), n)

    def tobf(x):
        return pltpu.bitcast(x, bf16)

    def pack(x):
        return pltpu.bitcast(x.astype(bf16), u32)

    def link(anchor, val):
        return val if anchor is None else jnp.where(pred, anchor, val)

    def lnk(anc, val):
        return val if anc is None else link(jnp.concatenate(anc, axis=0), val)

    def kv_stage(i):
        r0 = i * TM
        for c in range(LT):
            cs = slice(c * 128, (c + 1) * 128)
            k32[c, 8 + r0:8 + r0 + TM, :] = kb[r0:r0 + TM, cs].astype(f32)

    def kv_task(i, t, anc, direct=False):
        r0 = i * TM + 16 * t
        for c in range(LT):
            cs = slice(c * 128, (c + 1) * 128)
            hal = []
            for u in range(2):
                ra = 8 + r0 + 8 * u
                ksh = k32[c, ra:ra + 8, :] * skb[0, :, cs]
                if u == 0 and anc is not None:
                    ksh = link(anc[c], ksh)
                for j in range(1, 4):
                    ksh = ksh + k32[c, ra - j:ra - j + 8, :] * skb[j, :, cs]
                hal.append(ksh)
            kv = jnp.concatenate(hal, axis=0) * vb[r0:r0 + 16, cs].astype(f32)
            kvp[slice(r0 // 2, r0 // 2 + 8) if direct else drow(r0 // 2, 8), cs] = pack(kv)

    def store3(ref, j, vals, opaque, c0=0, nc=LT):
        for gq in range(NG):
            rs = drow(GR * gq, GR) if opaque else slice(GR * gq, GR * (gq + 1))
            for n, v in enumerate(vals):
                for c in range(nc):
                    ref[c0 + c, j, n, rs, :] = v[gq][:, 128 * c:128 * (c + 1)]

    def fwd_x(j, opaque=False):
        X = jnp.dot(tobf(tab[0:128, :]), tobf(kvp[j * 64:(j + 1) * 64, :]), preferred_element_type=f32)
        X4 = X.reshape(NG, 2, GR, D)
        a = X4[:, 0]; b = X4[:, 1]
        store3(xs, j, (a, b, a + b), opaque)
        return X

    def fwd_h(j, opaque=False, c0=0, nc=LT):
        fh = tobf(tab[128:256, :])
        ds_ = slice(128 * c0, 128 * (c0 + nc))
        H = jax.lax.dot_general(fh, hb[ds_, j * B:(j + 1) * B], NT, preferred_element_type=f32)
        H0 = H
        if j == 0:
            H = H + fh[:, 0:1].astype(f32) * dvv[...].astype(f32).reshape(1, D)[:, ds_]
        H4 = H.reshape(NG, 2, GR, 128 * nc)
        c_ = H4[:, 0]; d_ = H4[:, 1]
        store3(gs, j, (c_, d_ - c_, c_ + d_), opaque, c0, nc)
        return H0

    def touched(Sx, r, gi):
        for rr in range(r + 1):
            for gj, grp in enumerate(ASSIGN[rr][1]):
                if grp[0][1] == Sx and (rr < r or gj < gi):
                    return True
        return False

    def mac_group(work, g, hf, anc, use_acc):
        rs = slice(32 * g, 32 * (g + 1))
        xc, gc = {}, {}

        def X(j, c):
            if (j, c) not in xc:
                xc[(j, c)] = xs[hf, j, c, rs, :]
            return xc[(j, c)]

        def G(m, c):
            if (m, c) not in gc:
                gc[(m, c)] = gs[hf, m, c, rs, :]
            return gc[(m, c)]
        out = {}
        for s, js in work.items():
            s1 = s2 = s3 = None
            for j in js:
                m = s - j
                p1 = G(m, 0) * X(j, 2)
                p2 = G(m, 1) * X(j, 0)
                p3 = G(m, 2) * X(j, 1)
                if s1 is None:
                    s1, s2, s3 = lnk(anc, p1), p2, p3
                else:
                    s1, s2, s3 = s1 + p1, s2 + p2, s3 + p3
            re, im = s1 - s3, s1 + s2
            if use_acc:
                re, im = re + zacc[hf, s, 0, rs, :], im + zacc[hf, s, 1, rs, :]
            out[s] = (re, im)
        return out

    def pre_task(group, use_acc, t, anc):
        g, hf = t // 4, t % 4
        rs = slice(32 * g, 32 * (g + 1))
        Sx = group[0][1]
        js = [j for (J, _) in group for j in (2 * J, 2 * J + 1)]
        out = mac_group({2 * Sx: js, 2 * Sx + 1: js}, g, hf, anc, use_acc)
        for s, (re, im) in out.items():
            zacc[hf, s, 0, rs, :] = re; zacc[hf, s, 1, rs, :] = im

    def fin_task(r, use_acc, t, anc):
        g, hf = t // 4, t % 4
        rs = slice(32 * g, 32 * (g + 1))
        ls = slice(128 * hf, 128 * (hf + 1))
        js = [j for (J, _) in ASSIGN[r][0] for j in (2 * J, 2 * J + 1)]
        s0, s1_ = 2 * r, 2 * r + 1
        out = mac_group({s0: js + [s0], s1_: js + [s0, s1_]}, g, hf, anc, use_acc)
        (z0r, z0i), (z1r, z1i) = out[s0], out[s1_]
        pos = g < 2
        if r > 0:
            pr, pi = zacc[hf, s0 - 1, 0, rs, :], zacc[hf, s0 - 1, 1, rs, :]
            o0r, o0i = (z0r - pi, z0i + pr) if pos else (z0r + pi, z0i - pr)
        else:
            o0r, o0i = z0r, z0i
        o1r, o1i = (z1r - z0i, z1i + z0r) if pos else (z1r + z0i, z1i - z0r)
        if r + 1 < NS:
            zacc[hf, s1_, 0, rs, :] = z1r; zacc[hf, s1_, 1, rs, :] = z1i
        for n, o in enumerate((o0r, o0i, o1r, o1i)):
            zp[drow(64 * n + 16 * g, 16), ls] = pack(o)

    def inv_mm():
        ci = tobf(tab[256:288, :]); si = tobf(tab[288:320, :])
        anc = []
        for t in range(2):
            for hf in range(2):
                ls = slice(256 * hf, 256 * (hf + 1))
                A = jnp.dot(ci, tobf(zp[128 * t:128 * t + 64, ls]), preferred_element_type=f32)
                Bm = jnp.dot(si, tobf(zp[128 * t + 64:128 * (t + 1), ls]), preferred_element_type=f32)
                hi = A - Bm
                lo = A + Bm
                for a in range(8):
                    ybuf[drow(t * B + 64 + 8 * a, 8), ls] = hi[8 * a:8 * (a + 1)]
                    ybuf[drow(t * B + 8 * (7 - a), 8), ls] = lo[8 * a:8 * (a + 1)]
                anc += anchors(Bm, "row")
        return anc

    def wide(s):
        return jnp.concatenate([s] * LT, axis=1)

    def bc(s):
        return jnp.broadcast_to(s, (32, 128))

    def sl(t, n=32):
        return slice(n * t, n * (t + 1))

    def lnA_task(i, t, anc):
        r0 = i * TM + 32 * t
        x = qb[r0:r0 + 32, :].astype(f32)
        x = jnp.concatenate([lnk(anc, x[:, 0:128]), x[:, 128:]], axis=1)
        st_m[drow(32 * t, 32), :] = bc(jnp.mean(x, axis=-1, keepdims=True))

    def lnB_task(i, t, anc):
        r0 = i * TM + 32 * t
        x = qb[r0:r0 + 32, :].astype(f32)
        xc = x - wide(lnk(anc, st_m[sl(t), :]))
        xcb[drow(32 * t, 32), :] = xc
        v = jnp.mean(xc * xc, axis=-1, keepdims=True)
        st_r[drow(32 * t, 32), :] = bc(jax.lax.rsqrt(v + EPS))

    def lnC_task(i, t, anc):
        r0 = i * TM + 32 * t
        ys = []
        for u in range(4):
            y = ybuf[sl(4 * t + u, 8), :]
            if (32 * t) % B < 64:
                idx = 7 - jax.lax.broadcasted_iota(jnp.int32, (8, D), 0)
                y = jnp.take_along_axis(y, idx, axis=0)
            ys.append(y)
        y = jnp.concatenate(ys, axis=0)
        rr = wide(lnk(anc, st_r[sl(t), :]))
        m = st_m[sl(t), :]
        hc = xcb[sl(t), :] * (1.0 + rr * y)
        hres[drow(r0, 32), :] = hc + wide(m)
        mc = jnp.mean(hc, axis=-1, keepdims=True)
        v = jnp.maximum(jnp.mean(hc * hc, axis=-1, keepdims=True) - mc * mc, 0.0)
        st_m2[drow(32 * t, 32), :] = m + bc(mc)
        st_r2[drow(32 * t, 32), :] = bc(jax.lax.rsqrt(v + EPS))

    def lnE_task(i, t, anc):
        r0 = i * TM + 32 * t
        h = hres[r0:r0 + 32, :]
        xn = (h - wide(lnk(anc, st_m2[sl(t), :]))) * wide(st_r2[sl(t), :])
        xnp[drow(r0 // 2, 16), :] = pack(xn)

    def getw(wb, wp, c, first):
        lo, hi = FC[c]
        if first:
            w = wb[lo:hi, :]
            wp[lo // 2:hi // 2, :] = pltpu.bitcast(w, u32)
            return w
        return tobf(wp[lo // 2:hi // 2, :])

    def mm1c(i, c):
        lo, hi = FC[c]
        b1 = b1v[...].astype(f32).reshape(1, F)[:, lo:hi]
        xn = tobf(xnp[i * TM // 2:(i + 1) * TM // 2, :])
        h1 = jax.lax.dot_general(xn, getw(w1b, w1p, c, i == 0), NT, preferred_element_type=f32) + b1
        u = h1 * (GELU_C + (GELU_C * 0.044715) * (h1 * h1))
        g2 = h1 + h1 * jnp.tanh(u)
        gb = (gb0, gb1, gb2)[c]
        gb[drow(0, TM // 2), 0:hi - lo] = pack(g2)
        return anchors(h1[:, :(hi - lo) // 128 * 128], "col")

    def mm2c(i, c):
        lo, hi = FC[c]
        g = tobf((gb0, gb1, gb2)[c][:, 0:hi - lo])
        p = jnp.dot(g, getw(w2b, w2p, c, i == 0), preferred_element_type=f32)
        if c == 0:
            acc0[drow(0, TM), :] = p
        elif c == 1:
            acc1[drow(0, TM), :] = acc0[...] + p
        else:
            b2 = b2v[...].astype(f32).reshape(1, D)
            out = (acc1[...] + p) * 0.5 + (hres[i * TM:(i + 1) * TM, :] + b2)
            ob[i * TM:(i + 1) * TM, :] = out.astype(bf16)
            p = p[:, :384]
        return anchors(p, "col")

    def anchors(R, order):
        nr, nc = R.shape[0] // 8, R.shape[1] // 128
        if order == "col":
            idx = [(a, b) for b in range(nc) for a in range(nr)]
        else:
            idx = [(a, b) for a in range(nr) for b in range(nc)]
        return [(R, a, b) for a, b in idx]

    def run_region(steps, placements):
        phases = [ph for st in steps if st[0] == "mm" for ph in st[2]]
        names = [p[0] for p in phases]
        plan = {n: [] for n in names}
        load = [0.0] * len(phases)
        for tasks, cost, p_lo, p_hi in placements:
            idx = list(range(names.index(p_lo), names.index(p_hi) + 1))
            rem = [max(phases[k][2] - load[k], 1.0) for k in idx]
            tot = sum(rem)
            n = 4 * len(tasks)
            for ti, task in enumerate(tasks):
                anc = []
                for u in range(4):
                    x = (ti * 4 + u) / n * tot
                    for k, rk in zip(idx, rem):
                        if x < rk:
                            break
                        x -= rk
                    anc.append((k, min(int(x / rk * phases[k][1]), phases[k][1] - 1)))
                plan[names[max(a[0] for a in anc)]].append((task, anc))
            for k, rk in zip(idx, rem):
                load[k] += cost * len(tasks) * rk / tot
        res = {}
        for st in steps:
            if st[0] == "do":
                st[1]()
                continue
            A = st[1]()
            step = len(A) // sum(p[1] for p in st[2])
            A = A[::step]
            for name, na, _ in st[2]:
                res[names.index(name)] = A[:na]
                A = A[na:]
                for task, sel in plan[name]:
                    vals = []
                    for k, a_ in sel:
                        R, a, b = res[k][a_]
                        vals.append(R[8 * a:8 * (a + 1), 128 * b:128 * (b + 1)])
                    task(vals)

    def W(name):
        return ("do", P(wait, name))

    def C(i, c):
        ph = [[("c0", 128, 2230)], [("c1", 128, 2230)], [("c2a", 32, 830), ("c2b", 32, 830)]][c]
        return ("mm", P(mm1c, i, c), ph)

    def M(i, c):
        ph = [[("m0a", 100, 2560), ("m0b", 28, 720)], [("m1a", 64, 1580), ("m1b", 64, 1580)], [("m2", 96, 1860)]][c]
        return ("mm", P(mm2c, i, c), ph)

    def H(m, opaque=False, cap=HCAP):
        return ("mm", lambda: anchors(fwd_h(m, opaque), "row"), [("h%d" % m, 32, cap)])

    def Xf(j, opaque=False, cap=HCAP):
        return ("mm", lambda: anchors(fwd_x(j, opaque), "row"), [("x%d" % j, 32, cap)])

    INV = ("mm", inv_mm, [("inv", 64, 790)])

    def T(fn, n, *args):
        return [P(fn, *args, t) for t in range(n)]

    def ln_place(r, rng):
        return [(T(fn, 8, r), cost, a_, b_) for fn, cost, (a_, b_) in
                zip((lnA_task, lnB_task, lnC_task, lnE_task), (40, 100, 150, 45), rng)]

    def mac_place(r, fin_lo, fin_hi, pre_lo, pre_hi):
        fu, pgs = ASSIGN[r]
        out = []
        early = [gi for gi, grp in enumerate(pgs) if grp[0][1] == r]
        for gi in early:
            out.append((T(pre_task, 16, pgs[gi], touched(r, r, gi)), 96 * len(pgs[gi]) + 40, "c0", "c0"))
        out.append((T(fin_task, 16, r, touched(r, r, 99)), 132 + 96 * len(fu), "c1" if early else fin_lo, fin_hi))
        late = [(T(pre_task, 16, grp, touched(grp[0][1], r, gi)), 96 * len(grp) + 40, pre_lo, pre_hi)
                for gi, grp in enumerate(pgs) if gi not in early]
        return out, late

    def region(r):
        i = r - 1
        if r == 0:
            for c in range(LT):
                k32[c, 0:8, :] = jnp.zeros((8, 128), f32)
            wait("a")
            sk = skv[...].astype(f32)
            for j in range(4):
                skb[j] = jnp.broadcast_to(sk[j:j + 1, :], (8, D))
            kv_stage(0)
            for t in range(16):
                kv_task(0, t, None, direct=True)
            fwd_x(0, True); fwd_x(1, True)
            wait("b")
            for hh in range(2):
                fwd_h(0, False, 2 * hh, 2); fwd_h(1, False, 2 * hh, 2)
                for t in range(16):
                    if (t % 4) // 2 == hh:
                        fin_task(0, False, t, None)
            wait("q0")
            for t in range(8):
                lnA_task(0, t, None)
            steps = [INV]
            run_region(steps, [(T(lnB_task, 8, 0), 100, "inv", "inv")])
            for fn in (lnC_task, lnE_task):
                for t in range(8):
                    fn(0, t, None)
            return
        if r >= 2:
            cp_o[r - 2].start()
        if r == 1:
            steps = [W("w1c0"), C(i, 0), W("c"), ("do", P(kv_stage, 1)), H(2, True), H(3, True), Xf(2, True), Xf(3, True),
                     W("w1c1"), C(i, 1), W("w2c0"), W("w1c2"), M(i, 0), INV, C(i, 2), W("w2c1"), M(i, 1), M(i, 2)]
            m1, m2 = mac_place(r, "c1", "m0a", "m0b", "m2")
            pls = ([(T(kv_task, 16, 1), 75, "h2", "h2")] + m1
                   + ln_place(r, (("c1", "c1"), ("m0a", "m0b"), ("c2a", "c2b"), ("m1b", "m2"))) + m2)
        elif r == 2:
            steps = [W("d"), ("do", P(kv_stage, 2)), C(i, 0), H(4, True), H(5, True), Xf(4, True), Xf(5, True), C(i, 1), M(i, 0), INV,
                     W("e"), ("do", P(kv_stage, 3)), ("do", P(kv_stage, 4)), C(i, 2), M(i, 1), M(i, 2),
                     H(6), H(7), H(8), H(9), H(10), H(11), Xf(6), Xf(7, cap=1.0)]
            m1, m2 = mac_place(r, "c1", "m0a", "c1", "x6")
            pls = ([(T(kv_task, 16, 2), 75, "c0", "h4")] + m1
                   + ln_place(r, (("c0", "c0"), ("h4", "m0b"), ("c2a", "m1a"), ("m1b", "m2")))
                   + [(T(kv_task, 16, 3), 75, "m1a", "h9")] + m2)
        elif r < NS:
            steps = []
            if r == 3:
                steps += [W("f")]
            if r == 4:
                steps += [W("g")]
            if r + 2 < NS:
                steps += [("do", P(kv_stage, r + 2))]
            steps += [C(i, 0), C(i, 1), M(i, 0), INV, C(i, 2), M(i, 1), M(i, 2)]
            last = "m2"
            if r == 3:
                steps += [H(12), H(13), H(14), H(15)]
            if r + 1 < NS:
                steps += [Xf(2 * r + 2), Xf(2 * r + 3, cap=1.0)]
                last = "x%d" % (2 * r + 2)
            m1, m2 = mac_place(r, "c0", "m0a", "c0", last)
            pls = m1 + ln_place(r, (("c0", "c0"), ("c1", "m0b"), ("c2a", "m1a"), ("m1b", "m2")))
            if r + 1 < NS:
                pls += [(T(kv_task, 16, r + 1), 75, "c0", "m1b")]
            pls += m2
        else:
            steps = [C(i, 0), C(i, 1), M(i, 0), C(i, 2), M(i, 1), M(i, 2)]
            pls = []
        run_region(steps, pls)
        if r == NS:
            cp_o[NS - 1].start()
            for i in range(NS):
                cp_o[i].wait()

    only = list(range(NS + 1))
    blocks = [[0], [1], [2], [3], [4, 5], [6, 7, 8]]

    def block(rs):
        for r in rs:
            if r in only:
                region(r)
    for rs in blocks:
        if any(r in only for r in rs):
            pl.when(flag[rs[0]] == 0)(functools.partial(block, rs))


@jax.jit
def pallas_sequential_preLN__ssm_conv_h3__dense_activation_gelu__prompt_kernel(A_q, A_k, A_v, A_shift_k, A_ssm_k, A_ssm_D, B_x, B_w1, B_b1, B_w2, B_b2):
    tab = _consts()
    any_spec = pl.BlockSpec(memory_space=pl.ANY)
    bf16 = jnp.bfloat16
    f32 = jnp.float32
    u32 = jnp.uint32
    V = pltpu.VMEM
    out = pl.pallas_call(
        _kernel,
        out_shape=jax.ShapeDtypeStruct((S, D), bf16),
        in_specs=[any_spec] * 12,
        out_specs=any_spec,
        scratch_shapes=[
            pltpu.SMEM((16,), jnp.int32), V(tab.shape, u32),
            V((4, D), bf16), V((D,), bf16), V((F,), bf16), V((D,), bf16),
            V((S, D), bf16), V((S, D), bf16), V((S, D), bf16),
            V((D, S), bf16), V((F, D), bf16), V((F, D), bf16), V((F // 2, D), u32), V((F // 2, D), u32),
            V((S, D), bf16),
            V((LT, S + 8, 128), f32), V((4, 8, D), f32),
            V((LT, NB, 3, PR, 128), f32), V((LT, NB, 3, PR, 128), f32), V((LT, NB, 2, PR, 128), f32),
            V((S // 2, D), u32), V((S, D), f32), V((S // 2, D), u32),
            V((4 * B // 2, D), u32), V((TM, D), f32),
            V((TM // 2, 512), u32), V((TM // 2, 512), u32), V((TM // 2, 384), u32), V((TM, D), f32), V((TM, D), f32),
            V((TM, 128), f32), V((TM, 128), f32), V((TM, 128), f32), V((TM, 128), f32), V((TM, D), f32),
            pltpu.SemaphoreType.DMA((15,)),
        ],
        compiler_params=pltpu.CompilerParams(vmem_limit_bytes=110 * 1024 * 1024),
        name="h3ffn",
    )(jnp.asarray(np.zeros((16,), np.int32)), jnp.asarray(tab),
      A_q.reshape(S, D), A_k.reshape(S, D), A_v.reshape(S, D), A_shift_k.T, A_ssm_k, A_ssm_D,
      B_w1.T, B_b1, B_w2, B_b2)
    return out.reshape(1, S, D)
```

```python
import functools
import numpy as np
import jax
import jax.numpy as jnp
import jax.experimental.pallas as pl
import jax.experimental.pallas.tpu as pltpu

S, D, F = 2048, 512, 1376
TM = 256
NS = S // TM
HB = TM // 2
LT = D // 128
EPS = 1e-5
NT = (((1,), (1,)), ((), ()))
PR = TM + 8
FC = [(0, 512), (512, 1024), (1024, F)]
FR = F // 128 * 128
GELU_C = float(np.sqrt(2.0 / np.pi))
HCAP = 300.0
STARTS = (3, 4, 6)
GS = float((GELU_C * 0.044715) ** (1.0 / 3.0))

ASSIGN = {
    0: ([0], []),
    1: ([0, 1], []),
    2: ([0, 1, 2], []),
    3: ([0, 1, 2, 3], [(5, [0])]),
    4: ([0, 1, 2, 3, 4], [(6, [0, 1])]),
    5: ([1, 2, 3, 4, 5], [(7, [0, 1, 2])]),
    6: ([2, 3, 4, 5, 6], []),
    7: ([3, 4, 5, 6, 7], []),
}


def _kernel(flag_hbm, q_hbm, k_hbm, v_hbm, sk_hbm, h_hbm, dvec_hbm, w1_hbm, b1_hbm, w2_hbm, b2_hbm,
            o_hbm,
            flag, tab, skv, dvv, b1v, b2v, qb, kb, vb, hb, w1b, w2b, w1p, w2p, ob, k32, skb,
            xs, gs, zacc, kvp, hres, xnp, zp, ybuf, gb0, gb1, gb2, acc0, acc1, st_m, st_r, st_m2, st_r2, xcb, kvl, huw, b1c, sems):
    f32 = jnp.float32
    bf16 = jnp.bfloat16
    u32 = jnp.uint32
    P = functools.partial

    def rows(i):
        return pl.ds(i * TM, TM)

    def hcp(i):
        return (h_hbm.at[:, pl.ds(i * TM, TM)], hb.at[:, pl.ds(i * TM, TM)])

    def kcp(i):
        return (k_hbm.at[rows(i)], kb.at[rows(i)])

    def vcp(i):
        return (v_hbm.at[rows(i)], vb.at[rows(i)])

    def qcp(i):
        return (q_hbm.at[rows(i)], qb.at[rows(i)])

    def half(src, dst, hf):
        return (src.at[rows(0), pl.ds(256 * hf, 256)], dst.at[rows(0), pl.ds(256 * hf, 256)])

    def wcp(src, dst, c):
        lo, hi = FC[c]
        return (src.at[pl.ds(lo, hi - lo)], dst.at[pl.ds(lo, hi - lo)])

    groups = [
        ("a", [hcp(0), (dvec_hbm, dvv), (sk_hbm, skv)]),
        ("b0", [half(k_hbm, kb, 0), half(v_hbm, vb, 0)]),
        ("b1", [half(k_hbm, kb, 1), half(v_hbm, vb, 1)]),
        ("q0", [qcp(0)]),
        ("w1c0", [(b1_hbm, b1v), wcp(w1_hbm, w1b, 0)]),
        ("w1c1", [wcp(w1_hbm, w1b, 2)]),
        ("c", [hcp(1), kcp(1), vcp(1), wcp(w1_hbm, w1b, 1)]),
        ("w2c0", [(b2_hbm, b2v), wcp(w2_hbm, w2b, 0), qcp(1)]),
        ("w2c1", [wcp(w2_hbm, w2b, 1), wcp(w2_hbm, w2b, 2)]),
        ("d", [kcp(2), vcp(2), hcp(2), qcp(2)]),
        ("e", [kcp(3), vcp(3), hcp(3), hcp(4), hcp(5), kcp(4)]),
        ("f", [qcp(3), vcp(4), hcp(6), hcp(7), kcp(5)]),
        ("g", [qcp(4), vcp(5), qcp(5), kcp(6), vcp(6), qcp(6), kcp(7), vcp(7), qcp(7)]),
    ]
    cps = {name: [pltpu.make_async_copy(s, d, sems.at[gi]) for s, d in lst] for gi, (name, lst) in enumerate(groups)}
    nsem = len(groups)
    cp_flag = pltpu.make_async_copy(flag_hbm, flag, sems.at[nsem])
    cp_o = [pltpu.make_async_copy(ob.at[rows(i)], o_hbm.at[rows(i)], sems.at[nsem + 1]) for i in range(NS - 1)]

    tails = [(0, TM, 0, 128), (0, TM, 128, 128), (0, 128, 256, 256), (128, 64, 256, 256), (192, 64, 256, 256)]
    cp_t = [pltpu.make_async_copy(ob.at[pl.ds(S - TM + a, n), pl.ds(c, w)], o_hbm.at[pl.ds(S - TM + a, n), pl.ds(c, w)], sems.at[nsem + 1])
            for a, n, c, w in tails]

    def wait(name):
        for c in cps[name]:
            c.wait()

    def cis(idx):
        ang = (idx & 2047).astype(f32) * float(2.0 * np.pi / 2048.0)
        return jnp.cos(ang), jnp.sin(ang)

    def make_tables():
        i32 = jnp.int32
        lane8 = jax.lax.broadcasted_iota(i32, (8, 128), 1)
        row8 = jax.lax.broadcasted_iota(i32, (8, 128), 0)
        lane = jax.lax.broadcasted_iota(i32, (32, 128), 1)
        row = jax.lax.broadcasted_iota(i32, (32, 128), 0)
        rr, ri = cis(4 * row8 * (2 * lane8 + 1))
        kg, sec = row >> 2, row & 3
        kb0 = 16 * (kg & 3) + (kg >> 2)
        k0 = jnp.where(sec == 0, kb0, jnp.where(sec == 1, 127 - kb0, jnp.where(sec == 2, 255 - kb0, 128 + kb0)))
        tr, ti = cis((2 * k0 + 1) * (2 * lane + 1))
        for g in range(16):
            cs_, sn_ = [], []
            for n in (2 * g, 2 * g + 1):
                a, b = tr[n:n + 1], ti[n:n + 1]
                if (n & 3) in (0, 3):
                    cs_.append(a * rr - b * ri); sn_.append(-(a * ri) - b * rr)
                else:
                    cs_.append(a * rr + b * ri); sn_.append(a * ri - b * rr)
            tab[8 * g:8 * (g + 1), :] = pltpu.bitcast(jnp.concatenate(cs_, axis=0).astype(bf16), u32)
            tab[128 + 8 * g:128 + 8 * (g + 1), :] = pltpu.bitcast(jnp.concatenate(sn_, axis=0).astype(bf16), u32)

        def kb2(l):
            return 2 * (16 * ((l >> 4) & 3) + 2 * (l & 7) + (l >> 6)) + 1
        er, ei = cis(2 * kb2(lane8) * 4 * row8)
        cls, a_ = row >> 3, row & 7
        n1 = 32 * a_ + ((cls + 3) & 3) - (TM - 1)
        vr, vi = cis(2 * kb2(lane) * n1 + 512 * ((lane >> 3) & 1))
        vr, vi = vr * (1.0 / TM), vi * (1.0 / TM)
        for g in range(16):
            o = [vr[n:n + 1] * er - vi[n:n + 1] * ei for n in (2 * g, 2 * g + 1)]
            tab[256 + 8 * g:256 + 8 * (g + 1), :] = pltpu.bitcast(jnp.concatenate(o, axis=0).astype(bf16), u32)

    cp_flag.start()
    for name, _ in groups:
        for c in cps[name]:
            c.start()
    make_tables()
    cp_flag.wait()
    pred = flag[15] != 0
    zero = flag[14]
    zero8 = pl.multiple_of(zero, 8)

    def ov(ref):
        return ref.at[pl.ds(zero8 if len(ref.shape) == 2 else zero, ref.shape[0])]

    def rs_(start, n):
        return slice(start, start + n)

    def tobf(x):
        return pltpu.bitcast(x, bf16)

    def pack(x):
        return pltpu.bitcast(x.astype(bf16), u32)

    def link(anchor, val):
        return val if anchor is None else jax.lax.select(jnp.broadcast_to(pred, val.shape), anchor, val)

    def lnk(anc, val):
        return val if anc is None else link(jnp.concatenate(anc, axis=0), val)

    def kv_stage(i, cl=range(LT)):
        r0 = i * TM
        for c in cl:
            cs = slice(c * 128, (c + 1) * 128)
            k32[c, 8 + r0:8 + r0 + TM, :] = kb[r0:r0 + TM, cs].astype(f32)

    def stage_task(i, t, anc):
        r0 = i * TM + 32 * t
        for c in range(LT):
            cs = slice(c * 128, (c + 1) * 128)
            k32[c, 8 + r0:8 + r0 + 32, :] = link(jnp.concatenate([anc[c]] * 4, axis=0), kb[r0:r0 + 32, cs].astype(f32))

    def kv16(r0, c, anc):
        cs = slice(c * 128, (c + 1) * 128)
        ra = 8 + r0
        ksh = k32[c, ra:ra + 16, :] * skb[0, :, cs]
        if anc is not None:
            if anc[1]:
                ksh = link(jnp.concatenate([anc[0], anc[0]], axis=0), ksh)
            else:
                ksh = jnp.concatenate([link(anc[0], ksh[:8]), ksh[8:]], axis=0)
        for j in range(1, 4):
            ksh = ksh + k32[c, ra - j:ra - j + 16, :] * skb[j, :, cs]
        return ksh * vb[r0:r0 + 16, cs].astype(f32)

    def kvl_task(i, t, anc, cl=range(LT)):
        for c in cl:
            ov(kvl)[c, rs_(16 * t, 16), :] = kv16(i * TM + 16 * t, c, None if anc is None else (anc[c], True))

    def kvu_task(i, t, anc, direct=False, cl=range(LT)):
        idx = 7 - jax.lax.broadcasted_iota(jnp.int32, (8, 128), 0)
        for c in cl:
            cs = slice(c * 128, (c + 1) * 128)
            up = kv16(i * TM + HB + 16 * t, c, None if anc is None else (anc[c], False))
            lo = jnp.concatenate([jnp.take_along_axis(kvl[c, HB - 16 * t - 8 * (u + 1):HB - 16 * t - 8 * u, :], idx, axis=0)
                                  for u in range(2)], axis=0)
            for n, v in enumerate((up + lo, up - lo)):
                a = 64 * n + 8 * t
                (kvp if direct else ov(kvp))[rs_(a, 8), cs] = pack(v)

    def hf_task(j, t, anc, direct=False):
        idx = 127 - jax.lax.broadcasted_iota(jnp.int32, (16, 128), 1)
        for u in range(4):
            d0 = 64 * t + 16 * u
            lo = hb[d0:d0 + 16, j * TM:j * TM + HB].astype(f32)
            if anc is not None:
                lo = jnp.concatenate([link(anc[u], lo[:8]), lo[8:]], axis=0)
            lo = jnp.take_along_axis(lo, idx, axis=1)
            up = hb[d0:d0 + 16, j * TM + HB:(j + 1) * TM].astype(f32)
            for n, v in enumerate((up + lo, up - lo)):
                a = (j % 4) * (D // 2) + d0 // 2
                (huw if direct else ov(huw))[rs_(a, 8), 128 * n:128 * (n + 1)] = pack(v)

    def store3(ref, j, vals, opaque, c0):
        if opaque:
            ref = ov(ref)
        for n, v in enumerate(vals):
            for c in range(2):
                ref[c0 + c, j, n, 0:TM, :] = v[:, 128 * c:128 * (c + 1)]

    def fwd_x(j, hf, opaque=False, lean=False):
        ls = slice(256 * hf, 256 * (hf + 1))
        a = jnp.dot(tobf(tab[0:128, :]), tobf(kvp[0:64, ls]), preferred_element_type=f32)
        b = jnp.dot(tobf(tab[128:256, :]), tobf(kvp[64:128, ls]), preferred_element_type=f32)
        store3(xs, j, (a, b) if lean else (a, b, a + b), opaque, 2 * hf)
        return b

    def fwd_h(j, hf, opaque=False):
        cf = tobf(tab[0:128, :]); sf = tobf(tab[128:256, :])
        a = (j % 4) * (D // 2) + 128 * hf
        c_ = jax.lax.dot_general(cf, tobf(huw[a:a + 128, 0:128]), NT, preferred_element_type=f32)
        d_ = jax.lax.dot_general(sf, tobf(huw[a:a + 128, 128:256]), NT, preferred_element_type=f32)
        d0 = d_
        if j == 0:
            dv = dvv[...].astype(f32).reshape(1, D)[:, 256 * hf:256 * (hf + 1)]
            c_ = c_ + cf[:, HB - 1:HB].astype(f32) * dv
            d_ = d_ - sf[:, HB - 1:HB].astype(f32) * dv
        store3(gs, j, (c_, d_ - c_, c_ + d_), opaque, 2 * hf)
        return d0

    def touched(Sx, r):
        return any(s == Sx for rr in range(r) for s, _ in ASSIGN[rr][1])

    def mac(s, js, g, c, anc, use_acc, lean=0):
        rs = slice(32 * g, 32 * (g + 1))
        s1 = s2 = s3 = None
        for j in js:
            if lean:
                x2 = lnk(anc, xs[c, j, 0, rs, :]) + xs[c, j, 1, rs, :]
                anc = None
                if lean == 2:
                    xs[c, j, 2, rs, :] = x2
            else:
                x2 = xs[c, j, 2, rs, :]
            p1 = gs[c, s - j, 0, rs, :] * x2
            p2 = gs[c, s - j, 1, rs, :] * xs[c, j, 0, rs, :]
            p3 = gs[c, s - j, 2, rs, :] * xs[c, j, 1, rs, :]
            if s1 is None:
                s1, s2, s3 = lnk(anc, p1), p2, p3
            else:
                s1, s2, s3 = s1 + p1, s2 + p2, s3 + p3
        re, im = s1 - s3, s1 + s2
        if use_acc:
            re, im = re + zacc[c, s, 0, rs, :], im + zacc[c, s, 1, rs, :]
        return re, im

    def pre_task(s, js, use_acc, t, anc):
        g, c = t // 4, t % 4
        rs = slice(32 * g, 32 * (g + 1))
        re, im = mac(s, js, g, c, anc, use_acc, 2 if s == 0 else 0)
        zacc[c, s, 0, rs, :] = re; zacc[c, s, 1, rs, :] = im

    def fin_task(r, use_acc, t, anc):
        g, c = t // 4, t % 4
        rs = slice(32 * g, 32 * (g + 1))
        zr, zi = mac(r, ASSIGN[r][0], g, c, anc, use_acc, 1 if r == 0 else 0)
        if 0 < r < NS - 1:
            zacc[c, r, 0, rs, :] = zr; zacc[c, r, 1, rs, :] = zi
        q = []
        for sec in range(4):
            a, b = zr[8 * sec:8 * (sec + 1)], zi[8 * sec:8 * (sec + 1)]
            if r > 0:
                r8 = slice(32 * g + 8 * sec, 32 * g + 8 * (sec + 1))
                pr, pi = zacc[c, r - 1, 0, r8, :], zacc[c, r - 1, 1, r8, :]
                even = (g < 4) == (sec in (0, 3))
                a, b = (a - pi, b + pr) if even else (a + pi, b - pr)
            q.append((a, b))
        (ar, ai), (br, bi), (cr, ci), (dr, di) = q
        ppr, ppi, pmr, pmi = ar + cr, ai - ci, ar - cr, ai + ci
        qpr, qpi, qmr, qmi = dr + br, di - bi, dr - br, di + bi
        fs = ((ppr + qpr, ppi + qpi), (pmr - qmi, pmi + qmr), (ppr - qpr, ppi - qpi), (pmr + qmi, pmi - qmr))
        for n, (fr, fi) in enumerate(fs):
            ov(zp)[rs_(64 * n + 8 * g, 8), 128 * c:128 * (c + 1)] = pack(jnp.concatenate([fr, fi], axis=0))

    def inv_mm():
        anc = []
        for n in range(4):
            y = jnp.dot(tobf(tab[256 + 32 * n:288 + 32 * n, :]), tobf(zp[64 * n:64 * (n + 1), :]), preferred_element_type=f32)
            for c in range(LT):
                ov(ybuf)[c, pl.ds((n + 3) % 4, 64, stride=4), :] = y[:, 128 * c:128 * (c + 1)]
            anc += anchors(y, "row")[::2]
        return anc

    def mean(x):
        return jnp.sum(x, axis=-1, keepdims=True) * (1.0 / D)

    def wide(s):
        return jnp.concatenate([s] * LT, axis=1)

    def bc(s):
        return jnp.broadcast_to(s, (32, 128))

    def sl(t, n=32):
        return slice(n * t, n * (t + 1))

    def lnA_task(i, t, anc):
        r0 = i * TM + 32 * t
        x = qb[r0:r0 + 32, :].astype(f32)
        x = jnp.concatenate([lnk(anc, x[:, 0:128]), x[:, 128:]], axis=1)
        ov(st_m)[rs_(32 * t, 32), :] = bc(mean(x))

    def lnB_task(i, t, anc):
        r0 = i * TM + 32 * t
        x = qb[r0:r0 + 32, :].astype(f32)
        xc = x - wide(lnk(anc, st_m[sl(t), :]))
        ov(xcb)[rs_(32 * t, 32), :] = xc
        v = mean(xc * xc)
        ov(st_r)[rs_(32 * t, 32), :] = bc(jnp.exp(-0.5 * jnp.log(v + EPS)))

    def lnC_task(i, t, anc):
        r0 = i * TM + 32 * t
        y = jnp.concatenate([ybuf[c, sl(t), :] for c in range(LT)], axis=1)
        rr = wide(lnk(anc, st_r[sl(t), :]))
        m = st_m[sl(t), :]
        hc = xcb[sl(t), :] * (1.0 + rr * y)
        ov(hres)[rs_(r0, 32), :] = hc + wide(m)
        mc = mean(hc)
        v = jnp.maximum(mean(hc * hc) - mc * mc, 0.0)
        ov(st_m2)[rs_(32 * t, 32), :] = m + bc(mc)
        ov(st_r2)[rs_(32 * t, 32), :] = bc(jnp.exp(-0.5 * jnp.log((v + EPS) * (1.0 / (GS * GS)))))

    def lnE_task(i, t, anc, direct=False):
        r0 = i * TM + 32 * t
        h = hres[r0:r0 + 32, :]
        xn = (h - wide(lnk(anc, st_m2[sl(t), :]))) * wide(st_r2[sl(t), :])
        (xnp if direct else ov(xnp))[rs_(r0 // 2, 16), :] = pack(xn)

    def getw(wb, wp, lo, hi, first):
        if first:
            w = wb[lo:hi, :]
            wp[lo // 2:hi // 2, :] = pltpu.bitcast(w, u32)
            return w
        return tobf(wp[lo // 2:hi // 2, :])

    def gelu2(h1):
        return h1 + h1 * jnp.tanh(h1 * (GELU_C / GS + h1 * h1))

    def mm1c(i, c):
        lo, hi = FC[c]
        hi = min(hi, FR)
        b1 = b1v[...].astype(f32).reshape(1, F)[:, lo:hi] * GS
        xn = tobf(xnp[i * TM // 2:(i + 1) * TM // 2, :])
        h1 = jax.lax.dot_general(xn, getw(w1b, w1p, lo, hi, i == 0), NT, preferred_element_type=f32) + b1
        gb = (gb0, gb1, gb2)[c]
        ov(gb)[:, 0:hi - lo] = pack(gelu2(h1))
        return anchors(h1, "col")

    def mm1r(i):
        if i == 0:
            b1 = b1v[...].astype(f32).reshape(1, F)[:, F - 128:F] * GS
            b1c[...] = jnp.broadcast_to(b1, (128, 128)).T
        xn = tobf(xnp[i * TM // 2:(i + 1) * TM // 2, :])
        bc_ = b1c[128 - (F - FR):128, :]
        ht = jax.lax.dot_general(getw(w1b, w1p, FR, F, i == 0), xn, NT, preferred_element_type=f32) + jnp.concatenate([bc_, bc_], axis=1)
        gt = jnp.concatenate([gelu2(ht), jnp.zeros((128 - (F - FR), TM), f32)], axis=0)
        ov(gb2)[:, 256:384] = pack(gt.T)
        return anchors(ht, "col")

    def mm2c(i, c):
        lo, hi = FC[c]
        g = tobf((gb0, gb1, gb2)[c][:, 0:hi - lo])
        p = jnp.dot(g, getw(w2b, w2p, lo, hi, i == 0), preferred_element_type=f32)
        if c == 0:
            ov(acc0)[...] = p
        elif c == 1:
            ov(acc1)[...] = acc0[...] + p
        else:
            b2 = b2v[...].astype(f32).reshape(1, D)
            out = (acc1[...] + p) * (0.5 / GS) + (hres[i * TM:(i + 1) * TM, :] + b2)
            if i < NS - 1:
                ob[i * TM:(i + 1) * TM, :] = out.astype(bf16)
            else:
                for cc, (a, n, c0, w) in enumerate(tails):
                    ob[i * TM + a:i * TM + a + n, c0:c0 + w] = out[a:a + n, c0:c0 + w].astype(bf16)
                    cp_t[cc].start()
            p = p[:, :384]
        return anchors(p, "col")

    def anchors(R, order):
        nr, nc = R.shape[0] // 8, R.shape[1] // 128
        if order == "col":
            idx = [(a, b) for b in range(nc) for a in range(nr)]
        else:
            idx = [(a, b) for a in range(nr) for b in range(nc)]
        return [(R, a, b) for a, b in idx]

    def run_region(steps, placements):
        phases = [ph for st in steps if st[0] == "mm" for ph in st[2]]
        names = [p[0] for p in phases]
        plan = {n: [] for n in names}
        load = [0.0] * len(phases)
        for tasks, cost, p_lo, p_hi in placements:
            idx = list(range(names.index(p_lo), names.index(p_hi) + 1))
            rem = [max(phases[k][2] - load[k], 1.0) for k in idx]
            tot = sum(rem)
            n = 4 * len(tasks)
            for ti, task in enumerate(tasks):
                anc = []
                for u in range(4):
                    x = (ti * 4 + u) / n * tot
                    for k, rk in zip(idx, rem):
                        if x < rk:
                            break
                        x -= rk
                    anc.append((k, min(int(x / rk * phases[k][1]), phases[k][1] - 1)))
                plan[names[max(a[0] for a in anc)]].append((task, anc))
            for k, rk in zip(idx, rem):
                load[k] += cost * len(tasks) * rk / tot
        res = {}
        for st in steps:
            if st[0] == "do":
                st[1]()
                continue
            A = st[1]()
            step = len(A) // sum(p[1] for p in st[2])
            A = A[::step]
            for name, na, _ in st[2]:
                res[names.index(name)] = A[:na]
                A = A[na:]
                for task, sel in plan[name]:
                    vals = []
                    for k, a_ in sel:
                        R, a, b = res[k][a_]
                        vals.append(R[8 * a:8 * (a + 1), 128 * b:128 * (b + 1)])
                    task(vals)

    def W(name):
        return ("do", P(wait, name))

    def C(i, c):
        ph = [[("c0a", 64, 1115), ("c0b", 64, 1115)], [("c1", 128, 2230)], [("c2a", 32, 560), ("c2b", 32, 560)]][c]
        return ("mm", P(mm1c, i, c), ph)

    def M(i, c):
        ph = [[("m0a", 100, 2560), ("m0b", 28, 720)], [("m1a", 64, 1580), ("m1g", 24, 590), ("m1b", 40, 990)], [("m2a", 48, 930), ("m2b", 48, 930)]][c]
        return ("mm", P(mm2c, i, c), ph)

    def CR(i):
        return ("mm", P(mm1r, i), [("cr", 24, 400)])

    def C1(i):
        return ("mm", P(mm1c, i, 1), [("c1a", 64, 1115), ("c1b", 64, 1115)])

    def M1(i):
        return ("mm", P(mm2c, i, 1), [("m1x", 16, 400), ("m1y", 28, 700), ("m1z", 84, 2000)])

    def M0(i):
        return ("mm", P(mm2c, i, 0), [("m0x", 40, 1000), ("m0y", 60, 1500), ("m0b", 28, 720)])

    def H(m, opaque=False, cap=HCAP):
        return [("mm", lambda hf=hf: anchors(fwd_h(m, hf, opaque), "row"), [("h%d%s" % (m, "ab"[hf]), 32, cap)]) for hf in range(2)]

    def Xf(j, opaque=False, cap=HCAP):
        return [("mm", lambda hf=hf: anchors(fwd_x(j, hf, opaque), "row"), [("x%d%s" % (j, "ab"[hf]), 32, cap if hf == 0 else 1.0)])
                for hf in range(2)]

    INV = ("mm", inv_mm, [("inv", 64, 790)])

    def T(fn, n, *args):
        return [P(fn, *args, t) for t in range(n)]

    def ln_place(r, rng):
        return [(T(fn, 8, r), cost, a_, b_) for fn, cost, (a_, b_) in
                zip((lnA_task, lnB_task, lnC_task, lnE_task), (40, 100, 150, 45), rng)]

    def mac_place(r, fin_lo, fin_hi, pre_lo, pre_hi):
        fj, pgs = ASSIGN[r]
        out = [(T(fin_task, 32, r, touched(r, r)), 24 * len(fj) + 40, fin_lo, fin_hi)]
        late = [(T(pre_task, 32, s, js, touched(s, r)), 24 * len(js) + 8, pre_lo, pre_hi) for s, js in pgs]
        return out, late

    def kv_place(i, a_, b_, c_, d_):
        return [(T(kvl_task, 8, i), 80, a_, b_), (T(kvu_task, 8, i), 95, c_, d_)]

    def region(r):
        i = r - 1
        if r == 0:
            for c in range(LT):
                k32[c, 0:8, :] = jnp.zeros((8, 128), f32)
            wait("a")
            sk = skv[...].astype(f32)
            for j in range(4):
                skb[j] = jnp.broadcast_to(sk[j:j + 1, :], (16, D))
            for t in range(8):
                hf_task(0, t, None, direct=True)
            fwd_h(0, 0, True); fwd_h(0, 1, True)

            def kv0(hh):
                cl = (2 * hh, 2 * hh + 1)
                kv_stage(0, cl)
                for t in range(8):
                    kvl_task(0, t, None, cl)
                for t in range(8):
                    kvu_task(0, t, None, True, cl)

            def xf0(hh):
                fwd_x(0, hh, lean=True)
                for t in range(32):
                    if (t % 4) // 2 == hh:
                        fin_task(0, False, t, None)
            wait("b0")
            kv0(0)
            wait("b1")
            xf0(0)
            kv0(1)
            xf0(1)
            wait("q0")
            for t in range(8):
                lnA_task(0, t, None)
            run_region([INV], [(T(lnB_task, 8, 0), 100, "inv", "inv")])
            wait("w1c0")
            for t in range(8):
                lnC_task(0, t, None)
            for t in range(8):
                lnE_task(0, t, None, True)
            mm1c(0, 0)
            return
        if r == 4:
            cp_o[0].start(); cp_o[1].start()
        if r >= 4:
            cp_o[r - 2].start()
        if r == 1:
            steps = ([W("w1c1"), CR(i), C(i, 2), W("c"), ("do", P(kv_stage, 1)), C1(i)] + H(1, True) + Xf(1, True)
                     + [W("w2c0"), M0(i), W("w2c1"), INV, M1(i), M(i, 2)])
            m1, m2 = mac_place(r, "m0x", "m0b", "m0b", "m2b")
            pls = ([(T(pre_task, 32, 0, [0], False), 36, "cr", "c2b"), (T(hf_task, 8, 1), 45, "c1a", "c1a")] + kv_place(1, "c1a", "c1a", "c1b", "c1b") + m1
                   + ln_place(r, (("m0x", "m0y"), ("inv", "m1x"), ("m1z", "m1z"), ("m2b", "m2b"))) + m2)
        elif r == 2:
            steps = ([W("d"), ("do", P(kv_stage, 2)), CR(i), C(i, 0)] + H(2, True) + Xf(2, True) + [C(i, 1), M(i, 0),
                     W("e"), ("do", P(kv_stage, 3)), INV, C(i, 2), M(i, 1), M(i, 2)]
                     + H(3) + H(4) + H(5) + Xf(3)[:1])
            m1, m2 = mac_place(r, "c1", "m0b", "c1", "x3a")
            pls = ([(T(hf_task, 8, 2), 45, "c0a", "c0a")] + kv_place(2, "c0a", "c0a", "c0b", "c0b") + m1
                   + [(T(hf_task, 8, m), 45, "inv", "c2b") for m in (3, 4, 5)]
                   + ln_place(r, (("h2a", "x2a"), ("c1", "m0a"), ("m1a", "m1b"), ("m2b", "h3b")))
                   + kv_place(3, "c2a", "m1a", "m1g", "m2b") + m2 + [(T(stage_task, 8, 4), 35, "m1a", "m2b")])
        elif r < NS:
            steps = []
            if r == 3:
                steps += [W("f")]
            if r == 4:
                steps += [W("g")]
            if r in STARTS:
                steps += Xf(r, True)[1:]
            steps += [CR(i), C(i, 0), C(i, 1), M(i, 0), INV, C(i, 2), M(i, 1)]
            if r == 5:
                steps += Xf(r + 1)[:1]
            steps += [M(i, 2)]
            last = "m2b"
            if r == 3:
                steps += H(6) + H(7)
            if r + 1 < NS and r != 5:
                steps += Xf(r + 1)[:1] if r + 1 in STARTS else Xf(r + 1)
                last = "m2b" if r + 1 in STARTS else "x%da" % (r + 1)
            m1, m2 = mac_place(r, "cr", "m0a", "m0b", last)
            pls = [(T(hf_task, 8, m), 45, "c0a", "c0a") for m in (6, 7)] if r == 3 else []
            pls += m1 + ln_place(r, (("c0b", "c0b"), ("c1", "m0b"), ("c2a", "m1a"), ("m1b", "m2b" if r + 1 < NS else "m2a")))
            if r + 1 < NS:
                pls += kv_place(r + 1, "m0b", "c2b", "m1a", "m1g") if r == 5 else kv_place(r + 1, "m0b", "m1a", "m1g", "m2a")
            pls += m2
            if r + 2 < NS:
                pls += [(T(stage_task, 8, r + 2), 35, "c2a", "m2b")]
        else:
            steps = [CR(i), C(i, 0), C(i, 1), M(i, 0), C(i, 2), M(i, 1), M(i, 2)]
            pls = []
        run_region(steps, pls)
        if r == NS:
            for c in cp_o + cp_t:
                c.wait()

    only = list(range(NS + 1))
    blocks = [[0], [1], [2], [3], [4, 5], [6, 7, 8]]

    def block(rs):
        for r in rs:
            if r in only:
                region(r)
    for rs in blocks:
        if any(r in only for r in rs):
            pl.when(flag[rs[0]] == 0)(functools.partial(block, rs))


@jax.jit
def pallas_sequential_preLN__ssm_conv_h3__dense_activation_gelu__prompt_kernel(A_q, A_k, A_v, A_shift_k, A_ssm_k, A_ssm_D, B_x, B_w1, B_b1, B_w2, B_b2):
    any_spec = pl.BlockSpec(memory_space=pl.ANY)
    bf16 = jnp.bfloat16
    f32 = jnp.float32
    u32 = jnp.uint32
    V = pltpu.VMEM
    out = pl.pallas_call(
        _kernel,
        out_shape=jax.ShapeDtypeStruct((S, D), bf16),
        in_specs=[any_spec] * 11,
        out_specs=any_spec,
        scratch_shapes=[
            pltpu.SMEM((16,), jnp.int32), V((384, 128), u32),
            V((4, D), bf16), V((D,), bf16), V((F,), bf16), V((D,), bf16),
            V((S, D), bf16), V((S, D), bf16), V((S, D), bf16),
            V((D, S), bf16), V((F, D), bf16), V((F, D), bf16), V((F // 2, D), u32), V((F // 2, D), u32),
            V((S, D), bf16),
            V((LT, S + 8, 128), f32), V((4, 16, D), f32),
            V((LT, NS, 3, PR, 128), f32), V((LT, NS, 3, PR, 128), f32), V((LT, NS, 2, PR, 128), f32),
            V((TM // 2, D), u32), V((S, D), f32), V((S // 2, D), u32),
            V((TM, D), u32), V((LT, TM, 128), f32),
            V((TM // 2, 512), u32), V((TM // 2, 512), u32), V((TM // 2, 384), u32), V((TM, D), f32), V((TM, D), f32),
            V((TM, 128), f32), V((TM, 128), f32), V((TM, 128), f32), V((TM, 128), f32), V((TM, D), f32),
            V((LT, HB, 128), f32), V((4 * D // 2, 256), u32), V((128, 128), f32),
            pltpu.SemaphoreType.DMA((15,)),
        ],
        compiler_params=pltpu.CompilerParams(vmem_limit_bytes=110 * 1024 * 1024),
        name="h3ffn",
    )(jnp.asarray(np.zeros((16,), np.int32)),
      A_q.reshape(S, D), A_k.reshape(S, D), A_v.reshape(S, D), A_shift_k.T, A_ssm_k, A_ssm_D,
      B_w1.T, B_b1, B_w2, B_b2)
    return out.reshape(1, S, D)
```

```python
import functools
import numpy as np
import jax
import jax.numpy as jnp
import jax.experimental.pallas as pl
import jax.experimental.pallas.tpu as pltpu

S, D, F = 2048, 512, 1376
TM = 256
NS = S // TM
HB = TM // 2
LT = D // 128
EPS = 1e-5
NT = (((1,), (1,)), ((), ()))
PR = TM + 8
FC = [(0, 512), (512, 1024), (1024, F)]
FR = F // 128 * 128
GELU_C = float(np.sqrt(2.0 / np.pi))
HCAP = 300.0
NSEM = 5
STARTS = (3, 4, 6)
GS = float((GELU_C * 0.044715) ** (1.0 / 3.0))

ASSIGN = {
    0: ([0], []),
    1: ([0, 1], []),
    2: ([0, 1, 2], []),
    3: ([0, 1, 2, 3], [(5, [0])]),
    4: ([0, 1, 2, 3, 4], [(6, [0, 1])]),
    5: ([1, 2, 3, 4, 5], [(7, [0, 1, 2])]),
    6: ([2, 3, 4, 5, 6], []),
    7: ([3, 4, 5, 6, 7], []),
}


def _kernel(flag_hbm, q_hbm, k_hbm, v_hbm, sk_hbm, h_hbm, dvec_hbm, w1_hbm, b1_hbm, w2_hbm, b2_hbm,
            o_hbm,
            flag, tab, skv, dvv, b1v, b2v, qb, kb, vb, hb, w1b, w2b, w1p, w2p, ob, k32, skb,
            xs, gs, zacc, kvp, hres, xnp, zp, ybuf, gb0, gb1, gb2, acc0, acc1, st_m, st_r, st_m2, st_r2, xcb, kvl, huw, b1c, sems):
    f32 = jnp.float32
    bf16 = jnp.bfloat16
    u32 = jnp.uint32
    P = functools.partial

    def rows(i, n=1):
        return pl.ds(i * TM, n * TM)

    def hcp(i, n=1):
        return (h_hbm.at[:, rows(i, n)], hb.at[:, rows(i, n)])

    def kcp(i, n=1):
        return (k_hbm.at[rows(i, n)], kb.at[rows(i, n)])

    def vcp(i, n=1):
        return (v_hbm.at[rows(i, n)], vb.at[rows(i, n)])

    def qcp(i, n=1):
        return (q_hbm.at[rows(i, n)], qb.at[rows(i, n)])

    def half(src, dst, hf):
        return (src.at[rows(0), pl.ds(256 * hf, 256)], dst.at[rows(0), pl.ds(256 * hf, 256)])

    def wcp(src, dst, c):
        lo, hi = FC[c]
        return (src.at[pl.ds(lo, hi - lo)], dst.at[pl.ds(lo, hi - lo)])

    groups = [
        ("a", [hcp(0), (dvec_hbm, dvv), (sk_hbm, skv)]),
        ("b0", [half(k_hbm, kb, 0), half(v_hbm, vb, 0)]),
        ("b1", [half(k_hbm, kb, 1), half(v_hbm, vb, 1)]),
        ("q0", [qcp(0)]),
        ("w1c0", [(b1_hbm, b1v), wcp(w1_hbm, w1b, 0)]),
        ("w1c1", [wcp(w1_hbm, w1b, 2)]),
        ("c", [hcp(1), kcp(1), vcp(1), wcp(w1_hbm, w1b, 1)]),
        ("w2c0", [(b2_hbm, b2v), wcp(w2_hbm, w2b, 0), qcp(1)]),
        ("w2c1", [(w2_hbm.at[pl.ds(512, F - 512)], w2b.at[pl.ds(512, F - 512)])]),
        ("d", [kcp(2), vcp(2), hcp(2), qcp(2)]),
        ("e", [kcp(3, 2), vcp(3), hcp(3, 3)]),
        ("f", [qcp(3), vcp(4), hcp(6, 2), kcp(5)]),
        ("g", [qcp(4, 4), vcp(5, 3), kcp(6, 2)]),
    ]
    nsem = NSEM
    reuse = {groups[n][0]: groups[n - nsem][0] for n in range(nsem, len(groups))}
    semid = {name: gi % nsem for gi, (name, _) in enumerate(groups)}
    cps = {name: [pltpu.make_async_copy(s, d, sems.at[semid[name]]) for s, d in lst] for name, lst in groups}
    cp_flag = pltpu.make_async_copy(flag_hbm, flag, sems.at[nsem])
    cp_o = {r_: pltpu.make_async_copy(ob.at[rows(a_, n_)], o_hbm.at[rows(a_, n_)], sems.at[nsem])
            for r_, (a_, n_) in {4: (0, 3), 6: (3, 2), 7: (5, 1), 8: (6, 1)}.items()}

    tails = [(0, TM, 0, 128), (0, TM, 128, 128), (0, 128, 256, 256), (128, 64, 256, 256), (192, 64, 256, 256)]
    cp_t = [pltpu.make_async_copy(ob.at[pl.ds(S - TM + a, n), pl.ds(c, w)], o_hbm.at[pl.ds(S - TM + a, n), pl.ds(c, w)], sems.at[nsem])
            for a, n, c, w in tails]

    def wait(name):
        for c in cps[name]:
            c.wait()
        for late, early in reuse.items():
            if early == name:
                for c in cps[late]:
                    c.start()

    def cis(idx):
        ang = (idx & 2047).astype(f32) * float(2.0 * np.pi / 2048.0)
        return jnp.cos(ang), jnp.sin(ang)

    def make_tables():
        i32 = jnp.int32
        lane8 = jax.lax.broadcasted_iota(i32, (8, 128), 1)
        row8 = jax.lax.broadcasted_iota(i32, (8, 128), 0)
        lane = jax.lax.broadcasted_iota(i32, (32, 128), 1)
        row = jax.lax.broadcasted_iota(i32, (32, 128), 0)
        rr, ri = cis(4 * row8 * (2 * lane8 + 1))
        kg, sec = row >> 2, row & 3
        kb0 = 16 * (kg & 3) + (kg >> 2)
        k0 = jnp.where(sec == 0, kb0, jnp.where(sec == 1, 127 - kb0, jnp.where(sec == 2, 255 - kb0, 128 + kb0)))
        tr, ti = cis((2 * k0 + 1) * (2 * lane + 1))
        for g in range(16):
            cs_, sn_ = [], []
            for n in (2 * g, 2 * g + 1):
                a, b = tr[n:n + 1], ti[n:n + 1]
                if (n & 3) in (0, 3):
                    cs_.append(a * rr - b * ri); sn_.append(-(a * ri) - b * rr)
                else:
                    cs_.append(a * rr + b * ri); sn_.append(a * ri - b * rr)
            tab[8 * g:8 * (g + 1), :] = pltpu.bitcast(jnp.concatenate(cs_, axis=0).astype(bf16), u32)
            tab[128 + 8 * g:128 + 8 * (g + 1), :] = pltpu.bitcast(jnp.concatenate(sn_, axis=0).astype(bf16), u32)

        def kb2(l):
            return 2 * (16 * ((l >> 4) & 3) + 2 * (l & 7) + (l >> 6)) + 1
        er, ei = cis(2 * kb2(lane8) * 4 * row8)
        cls, a_ = row >> 3, row & 7
        n1 = 32 * a_ + ((cls + 3) & 3) - (TM - 1)
        vr, vi = cis(2 * kb2(lane) * n1 + 512 * ((lane >> 3) & 1))
        vr, vi = vr * (1.0 / TM), vi * (1.0 / TM)
        for g in range(16):
            o = [vr[n:n + 1] * er - vi[n:n + 1] * ei for n in (2 * g, 2 * g + 1)]
            tab[256 + 8 * g:256 + 8 * (g + 1), :] = pltpu.bitcast(jnp.concatenate(o, axis=0).astype(bf16), u32)

    cp_flag.start()
    for name, _ in groups:
        if name not in reuse:
            for c in cps[name]:
                c.start()
    make_tables()
    cp_flag.wait()
    pred = flag[15] != 0
    zero = flag[14]
    zero8 = pl.multiple_of(zero, 8)

    def ov(ref):
        return ref.at[pl.ds(zero8 if len(ref.shape) == 2 else zero, ref.shape[0])]

    def rs_(start, n):
        return slice(start, start + n)

    def tobf(x):
        return pltpu.bitcast(x, bf16)

    def pack(x):
        return pltpu.bitcast(x.astype(bf16), u32)

    def link(anchor, val):
        return val if anchor is None else jax.lax.select(jnp.broadcast_to(pred, val.shape), anchor, val)

    def lnk(anc, val):
        return val if anc is None else link(jnp.concatenate(anc, axis=0), val)

    def kv_stage(i, cl=range(LT)):
        r0 = i * TM
        for c in cl:
            cs = slice(c * 128, (c + 1) * 128)
            k32[c, 8 + r0:8 + r0 + TM, :] = kb[r0:r0 + TM, cs].astype(f32)

    def stage_task(i, t, anc):
        r0 = i * TM + 32 * t
        for c in range(LT):
            cs = slice(c * 128, (c + 1) * 128)
            k32[c, 8 + r0:8 + r0 + 32, :] = link(jnp.concatenate([anc[c]] * 4, axis=0), kb[r0:r0 + 32, cs].astype(f32))

    def kv16(r0, c, anc):
        cs = slice(c * 128, (c + 1) * 128)
        ra = 8 + r0
        ksh = k32[c, ra:ra + 16, :] * skb[0, :, cs]
        if anc is not None:
            if anc[1]:
                ksh = link(jnp.concatenate([anc[0], anc[0]], axis=0), ksh)
            else:
                ksh = jnp.concatenate([link(anc[0], ksh[:8]), ksh[8:]], axis=0)
        for j in range(1, 4):
            ksh = ksh + k32[c, ra - j:ra - j + 16, :] * skb[j, :, cs]
        return ksh * vb[r0:r0 + 16, cs].astype(f32)

    def kvl_task(i, t, anc, cl=range(LT)):
        for c in cl:
            ov(kvl)[c, rs_(16 * t, 16), :] = kv16(i * TM + 16 * t, c, None if anc is None else (anc[c], True))

    def kvu_task(i, t, anc, direct=False, cl=range(LT)):
        idx = 7 - jax.lax.broadcasted_iota(jnp.int32, (8, 128), 0)
        for c in cl:
            cs = slice(c * 128, (c + 1) * 128)
            up = kv16(i * TM + HB + 16 * t, c, None if anc is None else (anc[c], False))
            lo = jnp.concatenate([jnp.take_along_axis(kvl[c, HB - 16 * t - 8 * (u + 1):HB - 16 * t - 8 * u, :], idx, axis=0)
                                  for u in range(2)], axis=0)
            for n, v in enumerate((up + lo, up - lo)):
                a = 64 * n + 8 * t
                (kvp if direct else ov(kvp))[rs_(a, 8), cs] = pack(v)

    def hf_task(j, t, anc, direct=False):
        idx = 127 - jax.lax.broadcasted_iota(jnp.int32, (16, 128), 1)
        for u in range(4):
            d0 = 64 * t + 16 * u
            lo = hb[d0:d0 + 16, j * TM:j * TM + HB].astype(f32)
            if anc is not None:
                lo = jnp.concatenate([link(anc[u], lo[:8]), lo[8:]], axis=0)
            lo = jnp.take_along_axis(lo, idx, axis=1)
            up = hb[d0:d0 + 16, j * TM + HB:(j + 1) * TM].astype(f32)
            for n, v in enumerate((up + lo, up - lo)):
                a = (j % 4) * (D // 2) + d0 // 2
                (huw if direct else ov(huw))[rs_(a, 8), 128 * n:128 * (n + 1)] = pack(v)

    def store3(ref, j, vals, opaque, c0):
        if opaque:
            ref = ov(ref)
        for n, v in enumerate(vals):
            for c in range(2):
                ref[c0 + c, j, n, 0:TM, :] = v[:, 128 * c:128 * (c + 1)]

    def fwd_x(j, hf, opaque=False, lean=False):
        ls = slice(256 * hf, 256 * (hf + 1))
        a = jnp.dot(tobf(tab[0:128, :]), tobf(kvp[0:64, ls]), preferred_element_type=f32)
        b = jnp.dot(tobf(tab[128:256, :]), tobf(kvp[64:128, ls]), preferred_element_type=f32)
        store3(xs, j, (a, b) if lean else (a, b, a + b), opaque, 2 * hf)
        return b

    def fwd_h(j, hf, opaque=False):
        cf = tobf(tab[0:128, :]); sf = tobf(tab[128:256, :])
        a = (j % 4) * (D // 2) + 128 * hf
        c_ = jax.lax.dot_general(cf, tobf(huw[a:a + 128, 0:128]), NT, preferred_element_type=f32)
        d_ = jax.lax.dot_general(sf, tobf(huw[a:a + 128, 128:256]), NT, preferred_element_type=f32)
        d0 = d_
        if j == 0:
            dv = dvv[...].astype(f32).reshape(1, D)[:, 256 * hf:256 * (hf + 1)]
            c_ = c_ + cf[:, HB - 1:HB].astype(f32) * dv
            d_ = d_ - sf[:, HB - 1:HB].astype(f32) * dv
        store3(gs, j, (c_, d_ - c_, c_ + d_), opaque, 2 * hf)
        return d0

    def touched(Sx, r):
        return any(s == Sx for rr in range(r) for s, _ in ASSIGN[rr][1])

    def mac(s, js, g, c, anc, use_acc, lean=0):
        rs = slice(32 * g, 32 * (g + 1))
        s1 = s2 = s3 = None
        for j in js:
            if lean:
                x2 = lnk(anc, xs[c, j, 0, rs, :]) + xs[c, j, 1, rs, :]
                anc = None
                if lean == 2:
                    xs[c, j, 2, rs, :] = x2
            else:
                x2 = xs[c, j, 2, rs, :]
            p1 = gs[c, s - j, 0, rs, :] * x2
            p2 = gs[c, s - j, 1, rs, :] * xs[c, j, 0, rs, :]
            p3 = gs[c, s - j, 2, rs, :] * xs[c, j, 1, rs, :]
            if s1 is None:
                s1, s2, s3 = lnk(anc, p1), p2, p3
            else:
                s1, s2, s3 = s1 + p1, s2 + p2, s3 + p3
        re, im = s1 - s3, s1 + s2
        if use_acc:
            re, im = re + zacc[c, s, 0, rs, :], im + zacc[c, s, 1, rs, :]
        return re, im

    def pre_task(s, js, use_acc, t, anc):
        g, c = t // 4, t % 4
        rs = slice(32 * g, 32 * (g + 1))
        re, im = mac(s, js, g, c, anc, use_acc, 2 if s == 0 else 0)
        zacc[c, s, 0, rs, :] = re; zacc[c, s, 1, rs, :] = im

    def fin_task(r, use_acc, t, anc):
        g, c = t // 4, t % 4
        rs = slice(32 * g, 32 * (g + 1))
        zr, zi = mac(r, ASSIGN[r][0], g, c, anc, use_acc, 1 if r == 0 else 0)
        if 0 < r < NS - 1:
            zacc[c, r, 0, rs, :] = zr; zacc[c, r, 1, rs, :] = zi
        q = []
        for sec in range(4):
            a, b = zr[8 * sec:8 * (sec + 1)], zi[8 * sec:8 * (sec + 1)]
            if r > 0:
                r8 = slice(32 * g + 8 * sec, 32 * g + 8 * (sec + 1))
                pr, pi = zacc[c, r - 1, 0, r8, :], zacc[c, r - 1, 1, r8, :]
                even = (g < 4) == (sec in (0, 3))
                a, b = (a - pi, b + pr) if even else (a + pi, b - pr)
            q.append((a, b))
        (ar, ai), (br, bi), (cr, ci), (dr, di) = q
        ppr, ppi, pmr, pmi = ar + cr, ai - ci, ar - cr, ai + ci
        qpr, qpi, qmr, qmi = dr + br, di - bi, dr - br, di + bi
        fs = ((ppr + qpr, ppi + qpi), (pmr - qmi, pmi + qmr), (ppr - qpr, ppi - qpi), (pmr + qmi, pmi - qmr))
        for n, (fr, fi) in enumerate(fs):
            ov(zp)[rs_(64 * n + 8 * g, 8), 128 * c:128 * (c + 1)] = pack(jnp.concatenate([fr, fi], axis=0))

    def inv_mm():
        anc = []
        for n in range(4):
            y = jnp.dot(tobf(tab[256 + 32 * n:288 + 32 * n, :]), tobf(zp[64 * n:64 * (n + 1), :]), preferred_element_type=f32)
            for c in range(LT):
                ov(ybuf)[c, pl.ds((n + 3) % 4, 64, stride=4), :] = y[:, 128 * c:128 * (c + 1)]
            anc += anchors(y, "row")[::2]
        return anc

    def mean(x):
        return jnp.sum(x, axis=-1, keepdims=True) * (1.0 / D)

    def wide(s):
        return jnp.concatenate([s] * LT, axis=1)

    def bc(s):
        return jnp.broadcast_to(s, (32, 128))

    def sl(t, n=32):
        return slice(n * t, n * (t + 1))

    def lnA_task(i, t, anc):
        r0 = i * TM + 32 * t
        x = qb[r0:r0 + 32, :].astype(f32)
        x = jnp.concatenate([lnk(anc, x[:, 0:128]), x[:, 128:]], axis=1)
        ov(st_m)[rs_(32 * t, 32), :] = bc(mean(x))

    def lnB_task(i, t, anc):
        r0 = i * TM + 32 * t
        x = qb[r0:r0 + 32, :].astype(f32)
        xc = x - wide(lnk(anc, st_m[sl(t), :]))
        ov(xcb)[rs_(32 * t, 32), :] = xc
        v = mean(xc * xc)
        ov(st_r)[rs_(32 * t, 32), :] = bc(jnp.exp(-0.5 * jnp.log(v + EPS)))

    def lnC_task(i, t, anc):
        r0 = i * TM + 32 * t
        y = jnp.concatenate([ybuf[c, sl(t), :] for c in range(LT)], axis=1)
        rr = wide(lnk(anc, st_r[sl(t), :]))
        m = st_m[sl(t), :]
        hc = xcb[sl(t), :] * (1.0 + rr * y)
        ov(hres)[rs_(r0, 32), :] = hc + wide(m)
        mc = mean(hc)
        v = jnp.maximum(mean(hc * hc) - mc * mc, 0.0)
        ov(st_m2)[rs_(32 * t, 32), :] = m + bc(mc)
        ov(st_r2)[rs_(32 * t, 32), :] = bc(jnp.exp(-0.5 * jnp.log((v + EPS) * (1.0 / (GS * GS)))))

    def lnE_task(i, t, anc, direct=False):
        r0 = i * TM + 32 * t
        h = hres[r0:r0 + 32, :]
        xn = (h - wide(lnk(anc, st_m2[sl(t), :]))) * wide(st_r2[sl(t), :])
        (xnp if direct else ov(xnp))[rs_(r0 // 2, 16), :] = pack(xn)

    def getw(wb, wp, lo, hi, first):
        if first:
            w = wb[lo:hi, :]
            wp[lo // 2:hi // 2, :] = pltpu.bitcast(w, u32)
            return w
        return tobf(wp[lo // 2:hi // 2, :])

    def gelu2(h1):
        return h1 + h1 * jnp.tanh(h1 * (GELU_C / GS + h1 * h1))

    def mm1c(i, c):
        lo, hi = FC[c]
        hi = min(hi, FR)
        b1 = b1v[...].astype(f32).reshape(1, F)[:, lo:hi] * GS
        xn = tobf(xnp[i * TM // 2:(i + 1) * TM // 2, :])
        h1 = jax.lax.dot_general(xn, getw(w1b, w1p, lo, hi, i == 0), NT, preferred_element_type=f32) + b1
        gb = (gb0, gb1, gb2)[c]
        ov(gb)[:, 0:hi - lo] = pack(gelu2(h1))
        return anchors(h1, "col")

    def mm1r(i):
        if i == 0:
            b1 = b1v[...].astype(f32).reshape(1, F)[:, F - 128:F] * GS
            b1c[...] = jnp.broadcast_to(b1, (128, 128)).T
        xn = tobf(xnp[i * TM // 2:(i + 1) * TM // 2, :])
        bc_ = b1c[128 - (F - FR):128, :]
        ht = jax.lax.dot_general(getw(w1b, w1p, FR, F, i == 0), xn, NT, preferred_element_type=f32) + jnp.concatenate([bc_, bc_], axis=1)
        gt = jnp.concatenate([gelu2(ht), jnp.zeros((128 - (F - FR), TM), f32)], axis=0)
        ov(gb2)[:, 256:384] = pack(gt.T)
        return anchors(ht, "col")

    def mm2c(i, c):
        lo, hi = FC[c]
        g = tobf((gb0, gb1, gb2)[c][:, 0:hi - lo])
        p = jnp.dot(g, getw(w2b, w2p, lo, hi, i == 0), preferred_element_type=f32)
        if c == 0:
            ov(acc0)[...] = p
        elif c == 1:
            ov(acc1)[...] = acc0[...] + p
        else:
            b2 = b2v[...].astype(f32).reshape(1, D)
            out = (acc1[...] + p) * (0.5 / GS) + (hres[i * TM:(i + 1) * TM, :] + b2)
            if i < NS - 1:
                ob[i * TM:(i + 1) * TM, :] = out.astype(bf16)
            else:
                for cc, (a, n, c0, w) in enumerate(tails):
                    ob[i * TM + a:i * TM + a + n, c0:c0 + w] = out[a:a + n, c0:c0 + w].astype(bf16)
                    cp_t[cc].start()
            p = p[:, :384]
        return anchors(p, "col")

    def anchors(R, order):
        nr, nc = R.shape[0] // 8, R.shape[1] // 128
        if order == "col":
            idx = [(a, b) for b in range(nc) for a in range(nr)]
        else:
            idx = [(a, b) for a in range(nr) for b in range(nc)]
        return [(R, a, b) for a, b in idx]

    def run_region(steps, placements):
        phases = [ph for st in steps if st[0] == "mm" for ph in st[2]]
        names = [p[0] for p in phases]
        plan = {n: [] for n in names}
        load = [0.0] * len(phases)
        for tasks, cost, p_lo, p_hi in placements:
            idx = list(range(names.index(p_lo), names.index(p_hi) + 1))
            rem = [max(phases[k][2] - load[k], 1.0) for k in idx]
            tot = sum(rem)
            n = 4 * len(tasks)
            for ti, task in enumerate(tasks):
                anc = []
                for u in range(4):
                    x = (ti * 4 + u) / n * tot
                    for k, rk in zip(idx, rem):
                        if x < rk:
                            break
                        x -= rk
                    anc.append((k, min(int(x / rk * phases[k][1]), phases[k][1] - 1)))
                plan[names[max(a[0] for a in anc)]].append((task, anc))
            for k, rk in zip(idx, rem):
                load[k] += cost * len(tasks) * rk / tot
        res = {}
        for st in steps:
            if st[0] == "do":
                st[1]()
                continue
            A = st[1]()
            step = len(A) // sum(p[1] for p in st[2])
            A = A[::step]
            for name, na, _ in st[2]:
                res[names.index(name)] = A[:na]
                A = A[na:]
                for task, sel in plan[name]:
                    vals = []
                    for k, a_ in sel:
                        R, a, b = res[k][a_]
                        vals.append(R[8 * a:8 * (a + 1), 128 * b:128 * (b + 1)])
                    task(vals)

    def W(name):
        return ("do", P(wait, name))

    def C(i, c):
        ph = [[("c0a", 64, 1115), ("c0b", 64, 1115)], [("c1", 128, 2230)], [("c2a", 32, 560), ("c2b", 32, 560)]][c]
        return ("mm", P(mm1c, i, c), ph)

    def M(i, c):
        ph = [[("m0a", 100, 2560), ("m0b", 28, 720)], [("m1a", 64, 1580), ("m1g", 24, 590), ("m1b", 40, 990)], [("m2a", 48, 930), ("m2b", 48, 930)]][c]
        return ("mm", P(mm2c, i, c), ph)

    def CR(i):
        return ("mm", P(mm1r, i), [("cr", 24, 400)])

    def C1(i):
        return ("mm", P(mm1c, i, 1), [("c1a", 64, 1115), ("c1b", 64, 1115)])

    def M1(i):
        return ("mm", P(mm2c, i, 1), [("m1x", 16, 400), ("m1y", 28, 700), ("m1z", 84, 2000)])

    def M0(i):
        return ("mm", P(mm2c, i, 0), [("m0x", 40, 1000), ("m0y", 60, 1500), ("m0b", 28, 720)])

    def H(m, opaque=False, cap=HCAP):
        return [("mm", lambda hf=hf: anchors(fwd_h(m, hf, opaque), "row"), [("h%d%s" % (m, "ab"[hf]), 32, cap)]) for hf in range(2)]

    def Xf(j, opaque=False, cap=HCAP):
        return [("mm", lambda hf=hf: anchors(fwd_x(j, hf, opaque), "row"), [("x%d%s" % (j, "ab"[hf]), 32, cap if hf == 0 else 1.0)])
                for hf in range(2)]

    INV = ("mm", inv_mm, [("inv", 64, 790)])

    def T(fn, n, *args):
        return [P(fn, *args, t) for t in range(n)]

    def ln_place(r, rng):
        return [(T(fn, 8, r), cost, a_, b_) for fn, cost, (a_, b_) in
                zip((lnA_task, lnB_task, lnC_task, lnE_task), (40, 100, 150, 45), rng)]

    def mac_place(r, fin_lo, fin_hi, pre_lo, pre_hi):
        fj, pgs = ASSIGN[r]
        out = [(T(fin_task, 32, r, touched(r, r)), 24 * len(fj) + 40, fin_lo, fin_hi)]
        late = [(T(pre_task, 32, s, js, touched(s, r)), 24 * len(js) + 8, pre_lo, pre_hi) for s, js in pgs]
        return out, late

    def kv_place(i, a_, b_, c_, d_):
        return [(T(kvl_task, 8, i), 80, a_, b_), (T(kvu_task, 8, i), 95, c_, d_)]

    def region(r):
        i = r - 1
        if r == 0:
            for c in range(LT):
                k32[c, 0:8, :] = jnp.zeros((8, 128), f32)
            wait("a")
            sk = skv[...].astype(f32)
            for j in range(4):
                skb[j] = jnp.broadcast_to(sk[j:j + 1, :], (16, D))
            for t in range(8):
                hf_task(0, t, None, direct=True)
            fwd_h(0, 0, True); fwd_h(0, 1, True)

            def kv0(hh):
                cl = (2 * hh, 2 * hh + 1)
                kv_stage(0, cl)
                for t in range(8):
                    kvl_task(0, t, None, cl)
                for t in range(8):
                    kvu_task(0, t, None, True, cl)

            def xf0(hh):
                fwd_x(0, hh, lean=True)
                for t in range(32):
                    if (t % 4) // 2 == hh:
                        fin_task(0, False, t, None)
            wait("b0")
            kv0(0)
            wait("b1")
            xf0(0)
            kv0(1)
            xf0(1)
            wait("q0")
            for t in range(8):
                lnA_task(0, t, None)
            run_region([INV], [(T(lnB_task, 8, 0), 100, "inv", "inv")])
            wait("w1c0")
            for t in range(8):
                lnC_task(0, t, None)
            for t in range(8):
                lnE_task(0, t, None, True)
            mm1c(0, 0)
            return
        if r in cp_o:
            cp_o[r].start()
        if r == 1:
            steps = ([W("w1c1"), CR(i), C(i, 2), W("c"), ("do", P(kv_stage, 1)), C1(i)] + H(1, True) + Xf(1, True)
                     + [W("w2c0"), M0(i), W("w2c1"), INV, M1(i), M(i, 2)])
            m1, m2 = mac_place(r, "m0x", "m0b", "m0b", "m2b")
            pls = ([(T(pre_task, 32, 0, [0], False), 36, "cr", "c2b"), (T(hf_task, 8, 1), 45, "c1a", "c1a")] + kv_place(1, "c1a", "c1a", "c1b", "c1b") + m1
                   + ln_place(r, (("m0x", "m0y"), ("inv", "m1x"), ("m1z", "m1z"), ("m2b", "m2b"))) + m2)
        elif r == 2:
            steps = ([W("d"), ("do", P(kv_stage, 2)), CR(i), C(i, 0)] + H(2, True) + Xf(2, True) + [C(i, 1), M(i, 0),
                     W("e"), ("do", P(kv_stage, 3)), INV, C(i, 2), M(i, 1), M(i, 2)]
                     + H(3) + H(4) + H(5) + Xf(3)[:1])
            m1, m2 = mac_place(r, "c1", "m0b", "c1", "x3a")
            pls = ([(T(hf_task, 8, 2), 45, "c0a", "c0a")] + kv_place(2, "c0a", "c0a", "c0b", "c0b") + m1
                   + [(T(hf_task, 8, m), 45, "inv", "c2b") for m in (3, 4, 5)]
                   + ln_place(r, (("h2a", "x2a"), ("c1", "m0a"), ("m1a", "m1b"), ("m2b", "h3b")))
                   + kv_place(3, "c2a", "m1a", "m1g", "m2b") + m2 + [(T(stage_task, 8, 4), 35, "m1a", "m2b")])
        elif r < NS:
            steps = []
            if r == 3:
                steps += [W("f")]
            if r == 4:
                steps += [W("g")]
            if r in STARTS:
                steps += Xf(r, True)[1:]
            steps += [CR(i), C(i, 0), C(i, 1), M(i, 0), INV, C(i, 2), M(i, 1)]
            if r == 5:
                steps += Xf(r + 1)[:1]
            steps += [M(i, 2)]
            last = "m2b"
            if r == 3:
                steps += H(6) + H(7)
            if r + 1 < NS and r != 5:
                steps += Xf(r + 1)[:1] if r + 1 in STARTS else Xf(r + 1)
                last = "m2b" if r + 1 in STARTS else "x%da" % (r + 1)
            m1, m2 = mac_place(r, "cr", "m0a", "m0b", last)
            pls = [(T(hf_task, 8, m), 45, "c0a", "c0a") for m in (6, 7)] if r == 3 else []
            pls += m1 + ln_place(r, (("c0b", "c0b"), ("c1", "m0b"), ("c2a", "m1a"), ("m1b", "m2b" if r + 1 < NS else "m2a")))
            if r + 1 < NS:
                pls += kv_place(r + 1, "m0b", "c2b", "m1a", "m1g") if r == 5 else kv_place(r + 1, "m0b", "m1a", "m1g", "m2a")
            pls += m2
            if r + 2 < NS:
                pls += [(T(stage_task, 8, r + 2), 35, "c2a", "m2b")]
        else:
            steps = [CR(i), C(i, 0), C(i, 1), M(i, 0), C(i, 2), M(i, 1), M(i, 2)]
            pls = []
        run_region(steps, pls)
        if r == NS:
            for c in list(cp_o.values()) + cp_t:
                c.wait()

    def block(rs):
        for r in rs:
            region(r)

    for rs in [[0], [1], [2], [3], [4, 5], [6, 7, 8]]:
        pl.when(flag[rs[0]] == 0)(functools.partial(block, rs))


@jax.jit
def pallas_sequential_preLN__ssm_conv_h3__dense_activation_gelu__prompt_kernel(A_q, A_k, A_v, A_shift_k, A_ssm_k, A_ssm_D, B_x, B_w1, B_b1, B_w2, B_b2):
    any_spec = pl.BlockSpec(memory_space=pl.ANY)
    bf16 = jnp.bfloat16
    f32 = jnp.float32
    u32 = jnp.uint32
    V = pltpu.VMEM
    out = pl.pallas_call(
        _kernel,
        out_shape=jax.ShapeDtypeStruct((S, D), bf16),
        in_specs=[any_spec] * 11,
        out_specs=any_spec,
        scratch_shapes=[
            pltpu.SMEM((16,), jnp.int32), V((384, 128), u32),
            V((4, D), bf16), V((D,), bf16), V((F,), bf16), V((D,), bf16),
            V((S, D), bf16), V((S, D), bf16), V((S, D), bf16),
            V((D, S), bf16), V((F, D), bf16), V((F, D), bf16), V((F // 2, D), u32), V((F // 2, D), u32),
            V((S, D), bf16),
            V((LT, S + 8, 128), f32), V((4, 16, D), f32),
            V((LT, NS, 3, PR, 128), f32), V((LT, NS, 3, PR, 128), f32), V((LT, NS, 2, PR, 128), f32),
            V((TM // 2, D), u32), V((S, D), f32), V((S // 2, D), u32),
            V((TM, D), u32), V((LT, TM, 128), f32),
            V((TM // 2, 512), u32), V((TM // 2, 512), u32), V((TM // 2, 384), u32), V((TM, D), f32), V((TM, D), f32),
            V((TM, 128), f32), V((TM, 128), f32), V((TM, 128), f32), V((TM, 128), f32), V((TM, D), f32),
            V((LT, HB, 128), f32), V((4 * D // 2, 256), u32), V((128, 128), f32),
            pltpu.SemaphoreType.DMA((NSEM + 1,)),
        ],
        compiler_params=pltpu.CompilerParams(vmem_limit_bytes=110 * 1024 * 1024),
        name="h3ffn",
    )(jnp.asarray(np.zeros((16,), np.int32)),
      A_q.reshape(S, D), A_k.reshape(S, D), A_v.reshape(S, D), A_shift_k.T, A_ssm_k, A_ssm_D,
      B_w1.T, B_b1, B_w2, B_b2)
    return out.reshape(1, S, D)
```

```python
import functools
import numpy as np
import jax
import jax.numpy as jnp
import jax.experimental.pallas as pl
import jax.experimental.pallas.tpu as pltpu

S, D, F = 2048, 512, 1376
TM = 256
NS = S // TM
HB = TM // 2
LT = D // 128
EPS = 1e-5
NT = (((1,), (1,)), ((), ()))
PR = TM + 8
FC = [(0, 512), (512, 1024), (1024, F)]
FR = F // 128 * 128
GELU_C = float(np.sqrt(2.0 / np.pi))
HCAP = 300.0
NSEM = 5
STARTS = (5,)
GS = float((GELU_C * 0.044715) ** (1.0 / 3.0))

ASSIGN = {
    0: ([0], []),
    1: ([0, 1], []),
    2: ([0, 1, 2], [(3, [1, 2])]),
    3: ([0, 3], []),
    4: ([0, 1, 2, 3, 4], [(5, [0]), (6, [1, 2])]),
    5: ([1, 2, 3, 4, 5], [(7, [2, 3, 4])]),
    6: ([0, 3, 4, 5, 6], []),
    7: ([0, 1, 5, 6, 7], []),
}


def _kernel(flag_hbm, q_hbm, k_hbm, v_hbm, sk_hbm, h_hbm, dvec_hbm, w1_hbm, b1_hbm, w2_hbm, b2_hbm,
            o_hbm,
            flag, tab, skv, dvv, b1v, b2v, qb, kb, vb, hb, w1b, w2b, w1p, w2p, ob, k32, skb,
            xs, gs, zacc, kvp, hres, xnp, zp, ybuf, gb0, gb1, gb2, acc0, acc1, st_m, st_r, st_m2, st_r2, xcb, kvl, huw, b1c, sems):
    f32 = jnp.float32
    bf16 = jnp.bfloat16
    u32 = jnp.uint32
    P = functools.partial

    def rows(i, n=1):
        return pl.ds(i * TM, n * TM)

    def hcp(i, n=1):
        return (h_hbm.at[:, rows(i, n)], hb.at[:, rows(i, n)])

    def kcp(i, n=1):
        return (k_hbm.at[rows(i, n)], kb.at[rows(i, n)])

    def vcp(i, n=1):
        return (v_hbm.at[rows(i, n)], vb.at[rows(i, n)])

    def qcp(i, n=1):
        return (q_hbm.at[rows(i, n)], qb.at[rows(i, n)])

    def half(src, dst, hf):
        return (src.at[rows(0), pl.ds(256 * hf, 256)], dst.at[rows(0), pl.ds(256 * hf, 256)])

    def wcp(src, dst, c):
        lo, hi = FC[c]
        return (src.at[pl.ds(lo, hi - lo)], dst.at[pl.ds(lo, hi - lo)])

    groups = [
        ("a", [hcp(0), (dvec_hbm, dvv), (sk_hbm, skv)]),
        ("b0", [half(k_hbm, kb, 0), half(v_hbm, vb, 0)]),
        ("b1", [half(k_hbm, kb, 1), half(v_hbm, vb, 1)]),
        ("q0", [qcp(0)]),
        ("w1c0", [(b1_hbm, b1v), wcp(w1_hbm, w1b, 0)]),
        ("w1c1", [wcp(w1_hbm, w1b, 2), hcp(1)]),
        ("c", [kcp(1), vcp(1), wcp(w1_hbm, w1b, 1)]),
        ("w2c0", [(b2_hbm, b2v), wcp(w2_hbm, w2b, 0), qcp(1)]),
        ("w2c1", [(w2_hbm.at[pl.ds(512, F - 512)], w2b.at[pl.ds(512, F - 512)])]),
        ("d", [kcp(2), vcp(2), hcp(2), qcp(2)]),
        ("e", [hcp(3, 3), kcp(3, 3), vcp(3, 3), qcp(3, 2)]),
        ("g", [hcp(6, 2), kcp(6, 2), vcp(6, 2), qcp(5, 3)]),
    ]
    nsem = NSEM
    reuse = {groups[n][0]: groups[n - nsem][0] for n in range(nsem, len(groups))}
    semid = {name: gi % nsem for gi, (name, _) in enumerate(groups)}
    cps = {name: [pltpu.make_async_copy(s, d, sems.at[semid[name]]) for s, d in lst] for name, lst in groups}
    cp_flag = pltpu.make_async_copy(flag_hbm, flag, sems.at[nsem])
    cp_o = {r_: pltpu.make_async_copy(ob.at[rows(a_, n_)], o_hbm.at[rows(a_, n_)], sems.at[nsem])
            for r_, (a_, n_) in {5: (0, 4), 7: (4, 2), 8: (6, 1)}.items()}

    tails = [(0, TM, 0, 128), (0, TM, 128, 128), (0, 128, 256, 256), (128, 64, 256, 256), (192, 64, 256, 256)]
    cp_t = [pltpu.make_async_copy(ob.at[pl.ds(S - TM + a, n), pl.ds(c, w)], o_hbm.at[pl.ds(S - TM + a, n), pl.ds(c, w)], sems.at[nsem])
            for a, n, c, w in tails]

    def wait(name):
        for c in cps[name]:
            c.wait()
        for late, early in reuse.items():
            if early == name:
                for c in cps[late]:
                    c.start()

    def cis(idx):
        ang = (idx & 2047).astype(f32) * float(2.0 * np.pi / 2048.0)
        return jnp.cos(ang), jnp.sin(ang)

    def make_tables():
        i32 = jnp.int32
        lane8 = jax.lax.broadcasted_iota(i32, (8, 128), 1)
        row8 = jax.lax.broadcasted_iota(i32, (8, 128), 0)
        lane = jax.lax.broadcasted_iota(i32, (32, 128), 1)
        row = jax.lax.broadcasted_iota(i32, (32, 128), 0)
        rr, ri = cis(4 * row8 * (2 * lane8 + 1))
        kg, sec = row >> 2, row & 3
        kb0 = 16 * (kg & 3) + (kg >> 2)
        k0 = jnp.where(sec == 0, kb0, jnp.where(sec == 1, 127 - kb0, jnp.where(sec == 2, 255 - kb0, 128 + kb0)))
        tr, ti = cis((2 * k0 + 1) * (2 * lane + 1))
        for g in range(16):
            cs_, sn_ = [], []
            for n in (2 * g, 2 * g + 1):
                a, b = tr[n:n + 1], ti[n:n + 1]
                if (n & 3) in (0, 3):
                    cs_.append(a * rr - b * ri); sn_.append(-(a * ri) - b * rr)
                else:
                    cs_.append(a * rr + b * ri); sn_.append(a * ri - b * rr)
            tab[8 * g:8 * (g + 1), :] = pltpu.bitcast(jnp.concatenate(cs_, axis=0).astype(bf16), u32)
            tab[128 + 8 * g:128 + 8 * (g + 1), :] = pltpu.bitcast(jnp.concatenate(sn_, axis=0).astype(bf16), u32)

        def kb2(l):
            return 2 * (16 * ((l >> 4) & 3) + 2 * (l & 7) + (l >> 6)) + 1
        er, ei = cis(2 * kb2(lane8) * 4 * row8)
        cls, a_ = row >> 3, row & 7
        n1 = 32 * a_ + ((cls + 3) & 3) - (TM - 1)
        vr, vi = cis(2 * kb2(lane) * n1 + 512 * ((lane >> 3) & 1))
        vr, vi = vr * (1.0 / TM), vi * (1.0 / TM)
        for g in range(16):
            o = [vr[n:n + 1] * er - vi[n:n + 1] * ei for n in (2 * g, 2 * g + 1)]
            tab[256 + 8 * g:256 + 8 * (g + 1), :] = pltpu.bitcast(jnp.concatenate(o, axis=0).astype(bf16), u32)

    cp_flag.start()
    for name, _ in groups:
        if name not in reuse:
            for c in cps[name]:
                c.start()
    make_tables()
    cp_flag.wait()
    pred = flag[15] != 0
    zero = flag[14]
    zero8 = pl.multiple_of(zero, 8)

    def ov(ref):
        return ref.at[pl.ds(zero8 if len(ref.shape) == 2 else zero, ref.shape[0])]

    def rs_(start, n):
        return slice(start, start + n)

    def tobf(x):
        return pltpu.bitcast(x, bf16)

    def pack(x):
        return pltpu.bitcast(x.astype(bf16), u32)

    def link(anchor, val):
        return val if anchor is None else jax.lax.select(jnp.broadcast_to(pred, val.shape), anchor, val)

    def lnk(anc, val):
        return val if anc is None else link(jnp.concatenate(anc, axis=0), val)

    def kv_stage(i, cl=range(LT)):
        r0 = i * TM
        for c in cl:
            cs = slice(c * 128, (c + 1) * 128)
            k32[c, 8 + r0:8 + r0 + TM, :] = kb[r0:r0 + TM, cs].astype(f32)

    def stage_task(i, t, anc):
        r0 = i * TM + 32 * t
        for c in range(LT):
            cs = slice(c * 128, (c + 1) * 128)
            k32[c, 8 + r0:8 + r0 + 32, :] = link(jnp.concatenate([anc[c]] * 4, axis=0), kb[r0:r0 + 32, cs].astype(f32))

    def kv16(r0, c, anc):
        cs = slice(c * 128, (c + 1) * 128)
        ra = 8 + r0
        ksh = k32[c, ra:ra + 16, :] * skb[0, :, cs]
        if anc is not None:
            if anc[1]:
                ksh = link(jnp.concatenate([anc[0], anc[0]], axis=0), ksh)
            else:
                ksh = jnp.concatenate([link(anc[0], ksh[:8]), ksh[8:]], axis=0)
        for j in range(1, 4):
            ksh = ksh + k32[c, ra - j:ra - j + 16, :] * skb[j, :, cs]
        return ksh * vb[r0:r0 + 16, cs].astype(f32)

    def kvl_task(i, t, anc, cl=range(LT)):
        for c in cl:
            ov(kvl)[c, rs_(16 * t, 16), :] = kv16(i * TM + 16 * t, c, None if anc is None else (anc[c], True))

    def kvu_task(i, t, anc, direct=False, cl=range(LT)):
        idx = 7 - jax.lax.broadcasted_iota(jnp.int32, (8, 128), 0)
        for c in cl:
            cs = slice(c * 128, (c + 1) * 128)
            up = kv16(i * TM + HB + 16 * t, c, None if anc is None else (anc[c], False))
            lo = jnp.concatenate([jnp.take_along_axis(kvl[c, HB - 16 * t - 8 * (u + 1):HB - 16 * t - 8 * u, :], idx, axis=0)
                                  for u in range(2)], axis=0)
            for n, v in enumerate((up + lo, up - lo)):
                a = 64 * n + 8 * t
                (kvp if direct else ov(kvp))[rs_(a, 8), cs] = pack(v)

    def hf_task(j, t, anc, direct=False):
        idx = 127 - jax.lax.broadcasted_iota(jnp.int32, (16, 128), 1)
        for u in range(4):
            d0 = 64 * t + 16 * u
            lo = hb[d0:d0 + 16, j * TM:j * TM + HB].astype(f32)
            if anc is not None:
                lo = jnp.concatenate([link(anc[u], lo[:8]), lo[8:]], axis=0)
            lo = jnp.take_along_axis(lo, idx, axis=1)
            up = hb[d0:d0 + 16, j * TM + HB:(j + 1) * TM].astype(f32)
            for n, v in enumerate((up + lo, up - lo)):
                a = (j % 4) * (D // 2) + d0 // 2
                (huw if direct else ov(huw))[rs_(a, 8), 128 * n:128 * (n + 1)] = pack(v)

    def store3(ref, j, vals, opaque, c0):
        if opaque:
            ref = ov(ref)
        for n, v in enumerate(vals):
            for c in range(2):
                ref[c0 + c, j, n, 0:TM, :] = v[:, 128 * c:128 * (c + 1)]

    def fwd_x(j, hf, opaque=False, lean=False):
        ls = slice(256 * hf, 256 * (hf + 1))
        a = jnp.dot(tobf(tab[0:128, :]), tobf(kvp[0:64, ls]), preferred_element_type=f32)
        b = jnp.dot(tobf(tab[128:256, :]), tobf(kvp[64:128, ls]), preferred_element_type=f32)
        store3(xs, j, (a, b) if lean else (a, b, a + b), opaque, 2 * hf)
        return b

    def fwd_h(j, hf, opaque=False):
        cf = tobf(tab[0:128, :]); sf = tobf(tab[128:256, :])
        a = (j % 4) * (D // 2) + 128 * hf
        c_ = jax.lax.dot_general(cf, tobf(huw[a:a + 128, 0:128]), NT, preferred_element_type=f32)
        d_ = jax.lax.dot_general(sf, tobf(huw[a:a + 128, 128:256]), NT, preferred_element_type=f32)
        d0 = d_
        if j == 0:
            dv = dvv[...].astype(f32).reshape(1, D)[:, 256 * hf:256 * (hf + 1)]
            c_ = c_ + cf[:, HB - 1:HB].astype(f32) * dv
            d_ = d_ - sf[:, HB - 1:HB].astype(f32) * dv
        store3(gs, j, (c_, d_ - c_, c_ + d_), opaque, 2 * hf)
        return d0

    def touched(Sx, r):
        return any(s == Sx for rr in range(r) for s, _ in ASSIGN[rr][1])

    def mac(s, js, g, c, anc, use_acc, lean=0):
        rs = slice(32 * g, 32 * (g + 1))
        s1 = s2 = s3 = None
        for j in js:
            if lean:
                x2 = lnk(anc, xs[c, j, 0, rs, :]) + xs[c, j, 1, rs, :]
                anc = None
                if lean == 2:
                    xs[c, j, 2, rs, :] = x2
            else:
                x2 = xs[c, j, 2, rs, :]
            p1 = gs[c, s - j, 0, rs, :] * x2
            p2 = gs[c, s - j, 1, rs, :] * xs[c, j, 0, rs, :]
            p3 = gs[c, s - j, 2, rs, :] * xs[c, j, 1, rs, :]
            if s1 is None:
                s1, s2, s3 = lnk(anc, p1), p2, p3
            else:
                s1, s2, s3 = s1 + p1, s2 + p2, s3 + p3
        re, im = s1 - s3, s1 + s2
        if use_acc:
            re, im = re + zacc[c, s, 0, rs, :], im + zacc[c, s, 1, rs, :]
        return re, im

    def pre_task(s, js, use_acc, t, anc):
        g, c = t // 4, t % 4
        rs = slice(32 * g, 32 * (g + 1))
        re, im = mac(s, js, g, c, anc, use_acc, 2 if s == 0 else 0)
        zacc[c, s, 0, rs, :] = re; zacc[c, s, 1, rs, :] = im

    def fin_task(r, use_acc, t, anc):
        g, c = t // 4, t % 4
        rs = slice(32 * g, 32 * (g + 1))
        zr, zi = mac(r, ASSIGN[r][0], g, c, anc, use_acc, 1 if r == 0 else 0)
        if 0 < r < NS - 1:
            zacc[c, r, 0, rs, :] = zr; zacc[c, r, 1, rs, :] = zi
        q = []
        for sec in range(4):
            a, b = zr[8 * sec:8 * (sec + 1)], zi[8 * sec:8 * (sec + 1)]
            if r > 0:
                r8 = slice(32 * g + 8 * sec, 32 * g + 8 * (sec + 1))
                pr, pi = zacc[c, r - 1, 0, r8, :], zacc[c, r - 1, 1, r8, :]
                even = (g < 4) == (sec in (0, 3))
                a, b = (a - pi, b + pr) if even else (a + pi, b - pr)
            q.append((a, b))
        (ar, ai), (br, bi), (cr, ci), (dr, di) = q
        ppr, ppi, pmr, pmi = ar + cr, ai - ci, ar - cr, ai + ci
        qpr, qpi, qmr, qmi = dr + br, di - bi, dr - br, di + bi
        fs = ((ppr + qpr, ppi + qpi), (pmr - qmi, pmi + qmr), (ppr - qpr, ppi - qpi), (pmr + qmi, pmi - qmr))
        for n, (fr, fi) in enumerate(fs):
            ov(zp)[rs_(64 * n + 8 * g, 8), 128 * c:128 * (c + 1)] = pack(jnp.concatenate([fr, fi], axis=0))

    def inv_mm():
        anc = []
        for n in range(4):
            y = jnp.dot(tobf(tab[256 + 32 * n:288 + 32 * n, :]), tobf(zp[64 * n:64 * (n + 1), :]), preferred_element_type=f32)
            for c in range(LT):
                ov(ybuf)[c, pl.ds((n + 3) % 4, 64, stride=4), :] = y[:, 128 * c:128 * (c + 1)]
            anc += anchors(y, "row")[::2]
        return anc

    def mean(x):
        return jnp.sum(x, axis=-1, keepdims=True) * (1.0 / D)

    def wide(s):
        return jnp.concatenate([s] * LT, axis=1)

    def bc(s):
        return jnp.broadcast_to(s, (32, 128))

    def sl(t, n=32):
        return slice(n * t, n * (t + 1))

    def lnA_task(i, t, anc):
        r0 = i * TM + 32 * t
        x = qb[r0:r0 + 32, :].astype(f32)
        x = jnp.concatenate([lnk(anc, x[:, 0:128]), x[:, 128:]], axis=1)
        ov(st_m)[rs_(32 * t, 32), :] = bc(mean(x))

    def lnB_task(i, t, anc):
        r0 = i * TM + 32 * t
        x = qb[r0:r0 + 32, :].astype(f32)
        xc = x - wide(lnk(anc, st_m[sl(t), :]))
        ov(xcb)[rs_(32 * t, 32), :] = xc
        v = mean(xc * xc)
        ov(st_r)[rs_(32 * t, 32), :] = bc(jnp.exp(-0.5 * jnp.log(v + EPS)))

    def lnC_task(i, t, anc):
        r0 = i * TM + 32 * t
        y = jnp.concatenate([ybuf[c, sl(t), :] for c in range(LT)], axis=1)
        rr = wide(lnk(anc, st_r[sl(t), :]))
        m = st_m[sl(t), :]
        hc = xcb[sl(t), :] * (1.0 + rr * y)
        ov(hres)[rs_(r0, 32), :] = hc + wide(m)
        mc = mean(hc)
        v = jnp.maximum(mean(hc * hc) - mc * mc, 0.0)
        ov(st_m2)[rs_(32 * t, 32), :] = m + bc(mc)
        ov(st_r2)[rs_(32 * t, 32), :] = bc(jnp.exp(-0.5 * jnp.log((v + EPS) * (1.0 / (GS * GS)))))

    def lnE_task(i, t, anc, direct=False):
        r0 = i * TM + 32 * t
        h = hres[r0:r0 + 32, :]
        xn = (h - wide(lnk(anc, st_m2[sl(t), :]))) * wide(st_r2[sl(t), :])
        (xnp if direct else ov(xnp))[rs_(r0 // 2, 16), :] = pack(xn)

    def getw(wb, wp, lo, hi, first):
        if first:
            w = wb[lo:hi, :]
            wp[lo // 2:hi // 2, :] = pltpu.bitcast(w, u32)
            return w
        return tobf(wp[lo // 2:hi // 2, :])

    def gelu2(h1):
        return h1 + h1 * jnp.tanh(h1 * (GELU_C / GS + h1 * h1))

    def mm1c(i, c):
        lo, hi = FC[c]
        hi = min(hi, FR)
        b1 = b1v[...].astype(f32).reshape(1, F)[:, lo:hi] * GS
        xn = tobf(xnp[i * TM // 2:(i + 1) * TM // 2, :])
        h1 = jax.lax.dot_general(xn, getw(w1b, w1p, lo, hi, i == 0), NT, preferred_element_type=f32) + b1
        gb = (gb0, gb1, gb2)[c]
        ov(gb)[:, 0:hi - lo] = pack(gelu2(h1))
        return anchors(h1, "col")

    def mm1r(i):
        if i == 0:
            b1 = b1v[...].astype(f32).reshape(1, F)[:, F - 128:F] * GS
            b1c[...] = jnp.broadcast_to(b1, (128, 128)).T
        xn = tobf(xnp[i * TM // 2:(i + 1) * TM // 2, :])
        bc_ = b1c[128 - (F - FR):128, :]
        ht = jax.lax.dot_general(getw(w1b, w1p, FR, F, i == 0), xn, NT, preferred_element_type=f32) + jnp.concatenate([bc_, bc_], axis=1)
        gt = jnp.concatenate([gelu2(ht), jnp.zeros((128 - (F - FR), TM), f32)], axis=0)
        ov(gb2)[:, 256:384] = pack(gt.T)
        return anchors(ht, "col")

    def mm2c(i, c):
        lo, hi = FC[c]
        g = tobf((gb0, gb1, gb2)[c][:, 0:hi - lo])
        p = jnp.dot(g, getw(w2b, w2p, lo, hi, i == 0), preferred_element_type=f32)
        if c == 0:
            ov(acc0)[...] = p
        elif c == 1:
            ov(acc1)[...] = acc0[...] + p
        else:
            b2 = b2v[...].astype(f32).reshape(1, D)
            out = (acc1[...] + p) * (0.5 / GS) + (hres[i * TM:(i + 1) * TM, :] + b2)
            if i < NS - 1:
                ob[i * TM:(i + 1) * TM, :] = out.astype(bf16)
            else:
                for cc, (a, n, c0, w) in enumerate(tails):
                    ob[i * TM + a:i * TM + a + n, c0:c0 + w] = out[a:a + n, c0:c0 + w].astype(bf16)
                    cp_t[cc].start()
            p = p[:, :384]
        return anchors(p, "col")

    def anchors(R, order):
        nr, nc = R.shape[0] // 8, R.shape[1] // 128
        if order == "col":
            idx = [(a, b) for b in range(nc) for a in range(nr)]
        else:
            idx = [(a, b) for a in range(nr) for b in range(nc)]
        return [(R, a, b) for a, b in idx]

    def run_region(steps, placements):
        phases = [ph for st in steps if st[0] == "mm" for ph in st[2]]
        names = [p[0] for p in phases]
        plan = {n: [] for n in names}
        load = [0.0] * len(phases)
        for tasks, cost, p_lo, p_hi in placements:
            idx = list(range(names.index(p_lo), names.index(p_hi) + 1))
            rem = [max(phases[k][2] - load[k], 1.0) for k in idx]
            tot = sum(rem)
            n = 4 * len(tasks)
            for ti, task in enumerate(tasks):
                anc = []
                for u in range(4):
                    x = (ti * 4 + u) / n * tot
                    for k, rk in zip(idx, rem):
                        if x < rk:
                            break
                        x -= rk
                    anc.append((k, min(int(x / rk * phases[k][1]), phases[k][1] - 1)))
                plan[names[max(a[0] for a in anc)]].append((task, anc))
            for k, rk in zip(idx, rem):
                load[k] += cost * len(tasks) * rk / tot
        res = {}
        for st in steps:
            if st[0] == "do":
                st[1]()
                continue
            A = st[1]()
            step = len(A) // sum(p[1] for p in st[2])
            A = A[::step]
            for name, na, _ in st[2]:
                res[names.index(name)] = A[:na]
                A = A[na:]
                for task, sel in plan[name]:
                    vals = []
                    for k, a_ in sel:
                        R, a, b = res[k][a_]
                        vals.append(R[8 * a:8 * (a + 1), 128 * b:128 * (b + 1)])
                    task(vals)

    def W(name):
        return ("do", P(wait, name))

    def C(i, c):
        ph = [[("c0a", 64, 1115), ("c0b", 64, 1115)], [("c1", 128, 2230)], [("c2a", 32, 560), ("c2b", 32, 560)]][c]
        return ("mm", P(mm1c, i, c), ph)

    def M(i, c):
        ph = [[("m0a", 100, 2560), ("m0b", 28, 720)], [("m1a", 64, 1580), ("m1g", 24, 590), ("m1b", 40, 990)], [("m2a", 48, 930), ("m2b", 48, 930)]][c]
        return ("mm", P(mm2c, i, c), ph)

    def CR(i):
        return ("mm", P(mm1r, i), [("cr", 24, 400)])

    def C1(i):
        return ("mm", P(mm1c, i, 1), [("c1a", 56, 1000), ("c1m", 48, 800), ("c1b", 24, 400)])

    def M1(i):
        return ("mm", P(mm2c, i, 1), [("m1x", 16, 400), ("m1y", 28, 700), ("m1z", 84, 2000)])

    def M0(i):
        return ("mm", P(mm2c, i, 0), [("m0x", 40, 1000), ("m0y", 60, 1500), ("m0b", 28, 720)])

    def H(m, opaque=False, cap=HCAP):
        return [("mm", lambda hf=hf: anchors(fwd_h(m, hf, opaque), "row"), [("h%d%s" % (m, "ab"[hf]), 32, cap)]) for hf in range(2)]

    def Xf(j, opaque=False, cap=HCAP):
        return [("mm", lambda hf=hf: anchors(fwd_x(j, hf, opaque), "row"), [("x%d%s" % (j, "ab"[hf]), 32, cap if hf == 0 else 1.0)])
                for hf in range(2)]

    INV = ("mm", inv_mm, [("inv", 64, 790)])

    def T(fn, n, *args):
        return [P(fn, *args, t) for t in range(n)]

    def ln_place(r, rng):
        return [(T(fn, 8, r), cost, a_, b_) for fn, cost, (a_, b_) in
                zip((lnA_task, lnB_task, lnC_task, lnE_task), (40, 100, 150, 45), rng)]

    def mac_place(r, fin_lo, fin_hi, pre_lo, pre_hi):
        fj, pgs = ASSIGN[r]
        out = [(T(fin_task, 32, r, touched(r, r)), 24 * len(fj) + 40, fin_lo, fin_hi)]
        late = [(T(pre_task, 32, s, js, touched(s, r)), 24 * len(js) + 8, pre_lo, pre_hi) for s, js in pgs]
        return out, late

    def kv_place(i, a_, b_, c_, d_):
        return [(T(kvl_task, 8, i), 80, a_, b_), (T(kvu_task, 8, i), 95, c_, d_)]

    def region(r):
        i = r - 1
        if r == 0:
            for c in range(LT):
                k32[c, 0:8, :] = jnp.zeros((8, 128), f32)
            wait("a")
            sk = skv[...].astype(f32)
            for j in range(4):
                skb[j] = jnp.broadcast_to(sk[j:j + 1, :], (16, D))
            for t in range(8):
                hf_task(0, t, None, direct=True)
            fwd_h(0, 0, True); fwd_h(0, 1, True)

            def kv0(hh):
                cl = (2 * hh, 2 * hh + 1)
                kv_stage(0, cl)
                for t in range(8):
                    kvl_task(0, t, None, cl)
                for t in range(8):
                    kvu_task(0, t, None, True, cl)

            def xf0(hh):
                fwd_x(0, hh, lean=True)
                for t in range(32):
                    if (t % 4) // 2 == hh:
                        fin_task(0, False, t, None)
            wait("b0")
            kv0(0)
            wait("b1")
            xf0(0)
            kv0(1)
            xf0(1)
            wait("q0")
            for t in range(8):
                lnA_task(0, t, None)
            run_region([INV], [(T(lnB_task, 8, 0), 100, "inv", "inv")])
            wait("w1c0")
            for t in range(8):
                lnC_task(0, t, None)
            for t in range(8):
                lnE_task(0, t, None, True)
            run_region([C(0, 0)], [(T(pre_task, 32, 0, [0], False), 36, "c0a", "c0b")])
            return
        if r in cp_o:
            cp_o[r].start()
        if r == 1:
            steps = ([W("w1c1"), CR(i), C(i, 2)] + H(1, True) + [W("c"), ("do", P(kv_stage, 1)), C1(i)] + Xf(1, True)
                     + [W("w2c0"), M0(i), W("w2c1"), INV, M1(i), M(i, 2)])
            m1, m2 = mac_place(r, "m0x", "m0b", "m0b", "m2b")
            pls = ([(T(hf_task, 8, 1), 45, "cr", "c2a")] + kv_place(1, "c1a", "c1a", "c1m", "c1m") + m1
                   + ln_place(r, (("m0x", "m0y"), ("inv", "m1x"), ("m1z", "m1z"), ("m2b", "m2b"))) + m2)
        elif r in (2, 3):
            steps = ([W("d" if r == 2 else "e"), ("do", P(kv_stage, r)), CR(i), C(i, 0)] + H(r, True) + Xf(r, True)
                     + [C1(i), M(i, 0), INV, C(i, 2), M(i, 1), M(i, 2)])
            if r == 3:
                steps += H(4, True) + H(5, True) + Xf(4)
            m1, m2 = mac_place(r, "c1a", "m0a", "m0b", "m2a")
            pls = ([(T(hf_task, 8, r), 45, "cr", "c0a")] + kv_place(r, "c0a", "c0a", "c0b", "c0b")
                   + [(T(hf_task, 8, m), 45, "h3b", "x3a") for m in ((4, 5) if r == 3 else ())] + m1
                   + ln_place(r, (("h2a", "x2a") if r == 2 else ("c1a", "c1a"), ("c1a" if r == 2 else "c1m", "m0a"),
                                  ("c2a", "m1a"), ("m1b", "m2b"))) + m2)
            if r == 3:
                pls += ([(T(stage_task, 8, 4), 35, "c1a", "m0a")] + kv_place(4, "m0b", "m1a", "m1g", "m2b")
                        + [(T(stage_task, 8, 5), 35, "c2a", "m2b")])
        elif r < NS:
            steps = []
            if r == 5:
                steps += [W("g")]
            if r in STARTS:
                steps += Xf(r, True)[1:]
            steps += [CR(i), C(i, 0), C(i, 1), M(i, 0), INV, C(i, 2), M(i, 1)]
            if r + 1 in STARTS:
                steps += Xf(r + 1)[:1]
            steps += [M(i, 2)]
            if r == 5:
                steps += H(6, True) + H(7, True)
            if r + 1 < NS and r + 1 not in STARTS:
                steps += Xf(r + 1)
            m1, m2 = mac_place(r, "cr", "m0a", "m0b", "m2b")
            pls = [(T(hf_task, 8, m), 45, "c0a", "c0a") for m in (6, 7)] + [(T(stage_task, 8, 6), 35, "cr", "c1")] if r == 5 else []
            pls += m1 + ln_place(r, (("c0b", "c0b"), ("c1", "m0b"), ("c2a", "m1a"), ("m1b", "m2b" if r + 1 < NS else "m2a")))
            if r + 1 < NS:
                pls += (kv_place(r + 1, "m0b", "c2b", "m1a", "m1g") if r + 1 in STARTS
                        else kv_place(r + 1, "m0b", "m1a", "m1g", "m2a"))
            pls += m2
            if r == 5:
                pls += [(T(stage_task, 8, 7), 35, "c2a", "m2b")]
        else:
            steps = [CR(i), C(i, 0), C(i, 1), M(i, 0), C(i, 2), M(i, 1), M(i, 2)]
            pls = []
        run_region(steps, pls)
        if r == NS:
            for c in list(cp_o.values()) + cp_t:
                c.wait()

    def block(rs):
        for r in rs:
            region(r)

    for rs in [[0], [1], [2], [3, 4], [5, 6, 7, 8]]:
        pl.when(flag[rs[0]] == 0)(functools.partial(block, rs))


@jax.jit
def pallas_sequential_preLN__ssm_conv_h3__dense_activation_gelu__prompt_kernel(A_q, A_k, A_v, A_shift_k, A_ssm_k, A_ssm_D, B_x, B_w1, B_b1, B_w2, B_b2):
    any_spec = pl.BlockSpec(memory_space=pl.ANY)
    bf16 = jnp.bfloat16
    f32 = jnp.float32
    u32 = jnp.uint32
    V = pltpu.VMEM
    out = pl.pallas_call(
        _kernel,
        out_shape=jax.ShapeDtypeStruct((S, D), bf16),
        in_specs=[any_spec] * 11,
        out_specs=any_spec,
        scratch_shapes=[
            pltpu.SMEM((16,), jnp.int32), V((384, 128), u32),
            V((4, D), bf16), V((D,), bf16), V((F,), bf16), V((D,), bf16),
            V((S, D), bf16), V((S, D), bf16), V((S, D), bf16),
            V((D, S), bf16), V((F, D), bf16), V((F, D), bf16), V((F // 2, D), u32), V((F // 2, D), u32),
            V((S, D), bf16),
            V((LT, S + 8, 128), f32), V((4, 16, D), f32),
            V((LT, NS, 3, PR, 128), f32), V((LT, NS, 3, PR, 128), f32), V((LT, NS, 2, PR, 128), f32),
            V((TM // 2, D), u32), V((S, D), f32), V((S // 2, D), u32),
            V((TM, D), u32), V((LT, TM, 128), f32),
            V((TM // 2, 512), u32), V((TM // 2, 512), u32), V((TM // 2, 384), u32), V((TM, D), f32), V((TM, D), f32),
            V((TM, 128), f32), V((TM, 128), f32), V((TM, 128), f32), V((TM, 128), f32), V((TM, D), f32),
            V((LT, HB, 128), f32), V((4 * D // 2, 256), u32), V((128, 128), f32),
            pltpu.SemaphoreType.DMA((NSEM + 1,)),
        ],
        compiler_params=pltpu.CompilerParams(vmem_limit_bytes=110 * 1024 * 1024),
        name="h3ffn",
    )(jnp.asarray(np.zeros((16,), np.int32)),
      A_q.reshape(S, D), A_k.reshape(S, D), A_v.reshape(S, D), A_shift_k.T, A_ssm_k, A_ssm_D,
      B_w1.T, B_b1, B_w2, B_b2)
    return out.reshape(1, S, D)
```
